```python
import jax
import jax.numpy as jnp

def _softmax(x, axis=-1):
    return jax.nn.softmax(x, axis=axis)
def _gelu(x):
    return jax.nn.gelu(x, approximate=True)
def _silu(x):
    return jax.nn.silu(x)
def _sigmoid(x):
    return jax.nn.sigmoid(x)
def _layernorm(x, axis=-1, eps=1e-5):
    m = jnp.mean(x, axis=axis, keepdims=True)
    v = jnp.var(x, axis=axis, keepdims=True)
    return (x - m) / jnp.sqrt(v + eps)
def _scatter_add(tgt, idx, src, axis=0):
    return tgt.at[idx].add(src)
def _segment_sum(src, seg, n):
    return jax.ops.segment_sum(src, seg, n)
class _Rng:
    def __init__(self, key):
        self._k = key
    def _next(self):
        self._k, sub = jax.random.split(self._k)
        return sub
    def normal(self, shape):
        return jax.random.normal(self._next(), shape, dtype=jnp.bfloat16)
    def randint(self, lo, hi, shape):
        return jax.random.randint(self._next(), shape, lo, hi, dtype=jnp.int32)
    def uniform(self, shape, lo=0.0, hi=1.0):
        return jax.random.uniform(self._next(), shape, jnp.bfloat16, lo, hi)
    def permutation(self, n):
        return jax.random.permutation(self._next(), n)


kernel_name = 'parallel_sum__ssm_conv_s5__moe_arch_mod__prompt'

def setup_inputs():
    _rng = _Rng(jax.random.key(int.from_bytes(__import__("os").urandom(4), "little")))
    _w = (lambda a: (lambda t: t.astype(jnp.bfloat16) if jnp.issubdtype(t.dtype, jnp.floating) else t)(jnp.asarray(a)))
    def _A_setup():
        B, S, D = 1, 2048, 1024
        P = D
        Lambda_re = -0.5 * jnp.exp((lambda *s: _rng.normal(s) * 0.05)(P))
        Lambda_im = (lambda *s: _rng.normal(s) * 0.05)(P) * 1.0
        B_re = (lambda *s: _rng.normal(s) * 0.05)(P, D) * (D ** -0.5)
        B_im = (lambda *s: _rng.normal(s) * 0.05)(P, D) * (D ** -0.5)
        C_re = (lambda *s: _rng.normal(s) * 0.05)(D, P) * (P ** -0.5)
        C_im = (lambda *s: _rng.normal(s) * 0.05)(D, P) * (P ** -0.5)
        log_dt = (lambda *s: _rng.normal(s) * 0.05)(P) * 0.3 - 2.0
        Dskip = (lambda *s: _rng.normal(s) * 0.05)(D)
        return {
            "x": _w((lambda *s: _rng.normal(s) * 0.05)(B, S, D)),
            "Lambda_re": _w(Lambda_re),
            "Lambda_im": _w(Lambda_im),
            "B_re": _w(B_re),
            "B_im": _w(B_im),
            "C_re": _w(C_re),
            "C_im": _w(C_im),
            "log_dt": _w(log_dt),
            "Dskip": _w(Dskip),
        }
    _A_in = _A_setup()

    def _B_setup():
        B, S, D, F, C = 1, 2048, 1024, 3584, 2
        return {
            "x": _w((lambda *s: _rng.normal(s) * 0.05)(B, S, D)),
            "w_r": _w((lambda *s: _rng.normal(s) * 0.05)(D)),
            "w_gate": _w((lambda *s: _rng.normal(s) * 0.05)(D, F)),
            "w_up": _w((lambda *s: _rng.normal(s) * 0.05)(D, F)),
            "w_down": _w((lambda *s: _rng.normal(s) * 0.05)(F, D)),
        }
    _B_in = _B_setup()

    return {
        "A_x": _A_in["x"],
        "A_Lambda_re": _A_in["Lambda_re"],
        "A_Lambda_im": _A_in["Lambda_im"],
        "A_B_re": _A_in["B_re"],
        "A_B_im": _A_in["B_im"],
        "A_C_re": _A_in["C_re"],
        "A_C_im": _A_in["C_im"],
        "A_log_dt": _A_in["log_dt"],
        "A_Dskip": _A_in["Dskip"],
        "B_x": _B_in["x"],
        "B_w_r": _B_in["w_r"],
        "B_w_gate": _B_in["w_gate"],
        "B_w_up": _B_in["w_up"],
        "B_w_down": _B_in["w_down"],
    }

def reference(A_x, A_Lambda_re, A_Lambda_im, A_B_re, A_B_im, A_C_re, A_C_im, A_log_dt, A_Dskip, B_x, B_w_r, B_w_gate, B_w_up, B_w_down):
    def _A_ref(x, Lambda_re, Lambda_im, B_re, B_im, C_re, C_im, log_dt, Dskip):
        Bsz, L, H = x.shape
        Lam = Lambda_re + 1j * Lambda_im
        Bmat = B_re + 1j * B_im
        Cmat = C_re + 1j * C_im
        dt = jnp.exp(log_dt)
        Lam_bar = jnp.exp(dt * Lam)
        B_bar = ((Lam_bar - 1.0) / Lam)[:, None] * Bmat
        Bu = jnp.einsum("bld,pd->blp", x + 0j, B_bar)
        h = jnp.zeros_like(Bu[:, 0, :])
        hs = []
        for t in range(L):
            h = Lam_bar[None, :] * h + Bu[:, t, :]
            hs.append(h)
        hseq = jnp.stack(hs, 1)
        y = 2.0 * jnp.einsum("blp,dp->bld", hseq, Cmat).real + x * Dskip[None, None, :]
        return y

    def _B_ref(x, w_r, w_gate, w_up, w_down):
        B, S, D = x.shape
        C = 2
        r = x @ w_r
        idx = jnp.argsort(-r, axis=-1)[:, :C]
        idx_e = jnp.repeat(idx.reshape(B, C, 1), D, axis=2)
        x_sel = jnp.take_along_axis(x, idx_e, axis=1)
        g = _silu(x_sel @ w_gate)
        u = x_sel @ w_up
        y = (g * u) @ w_down
        r_sel = _sigmoid(jnp.take_along_axis(r, idx, axis=1))
        y = y * r_sel.reshape(B, C, 1)
        b_off = (jnp.arange(B) * S).reshape(B, 1)
        flat_idx = (idx + b_off).reshape(B * C)
        zero = (x * 0.0).reshape(B * S, D)
        upd = _scatter_add(zero, flat_idx, y.reshape(B * C, D), axis=0)
        return x + upd.reshape(B, S, D)

    x = A_x
    xn = _layernorm(x, axis=-1)
    return x + _A_ref(xn, A_Lambda_re, A_Lambda_im, A_B_re, A_B_im, A_C_re, A_C_im, A_log_dt, A_Dskip) + _B_ref(xn, B_w_r, B_w_gate, B_w_up, B_w_down)
```

```python
import jax
import jax.numpy as jnp
from jax import lax
import jax.experimental.pallas as pl
import jax.experimental.pallas.tpu as pltpu

L, D, P, F = 2048, 1024, 1024, 3584
T = 256
J = T // 8
NB = L // T
G = P // 128
FC = 512
NF = F // FC
f32, bf16 = jnp.float32, jnp.bfloat16
NT = (((1,), (1,)), ((), ()))


def _rb(v):
    return v.astype(bf16).astype(f32)


def _kernel(x_hbm, lre_ref, lim_ref, bre_hbm, bim_hbm, cre_hbm, cim_hbm, ldt_ref, dsk_ref,
            wr_ref, wg_hbm, wu_hbm, wd_hbm, o_hbm,
            xb, xn, xp, ob, bw, cw, wg, wu, wd, bu0, bu1, h0, h1, rr, st, sem, osem):
    def cp(src, dst, k):
        return pltpu.make_async_copy(src, dst, sem.at[k])

    x_cp = [cp(x_hbm.at[pl.ds(i * T, T)], xb.at[pl.ds(i * T, T)], i) for i in range(NB)]
    b_cp = [cp(bre_hbm, bw.at[0], NB), cp(bim_hbm, bw.at[1], NB + 1)]
    c_cp = [cp(cre_hbm, cw.at[0], NB + 2), cp(cim_hbm, cw.at[1], NB + 3)]
    w_cp = [cp(wg_hbm, wg, NB + 4), cp(wu_hbm, wu, NB + 5), cp(wd_hbm, wd, NB + 6)]
    for c in x_cp + b_cp + c_cp + w_cp:
        c.start()

    lre = lre_ref[...].astype(f32)
    lim = lim_ref[...].astype(f32)
    dt = _rb(jnp.exp(ldt_ref[...].astype(f32)))
    ar, ai = dt * lre, dt * lim
    mag = jnp.exp(ar)
    lbr, lbi = mag * jnp.cos(ai), mag * jnp.sin(ai)
    den = lre * lre + lim * lim
    cfr = ((lbr - 1.0) * lre + lbi * lim) / den
    cfi = (lbi * lre - (lbr - 1.0) * lim) / den
    st[0] = jnp.broadcast_to(lbr, (8, P))
    st[1] = jnp.broadcast_to(lbi, (8, P))
    sub = lax.broadcasted_iota(jnp.int32, (8, P), 0)
    for k in range(3):
        n = float(J * (1 << k))
        m = jnp.exp(ar * n)
        keep = sub >= (1 << k)
        st[2 + 2 * k] = jnp.where(keep, jnp.broadcast_to(m * jnp.cos(ai * n), (8, P)), 0.0)
        st[3 + 2 * k] = jnp.where(keep, jnp.broadcast_to(m * jnp.sin(ai * n), (8, P)), 0.0)
    st[8] = jnp.zeros((8, P), f32)
    st[9] = jnp.zeros((8, P), f32)

    dsk = dsk_ref[...].astype(f32)
    wr = wr_ref[...].astype(f32)
    for i in range(NB):
        x_cp[i].wait()

        def ln(q, _):
            rows = pl.ds(pl.multiple_of(i * T + q * 32, 32), 32)
            x = xb[rows, :].astype(f32)
            mu = jnp.mean(x, axis=-1, keepdims=True)
            c = x - mu
            var = _rb(jnp.mean(c * c, axis=-1, keepdims=True))
            s = _rb(jnp.sqrt(_rb(var + 1e-5)))
            n = _rb(_rb(x - _rb(mu)) / s)
            base = x + _rb(n * dsk) + n
            for g in range(G):
                xn[g, rows, :] = n[:, g * 128:(g + 1) * 128]
                ob[g, rows, :] = base[:, g * 128:(g + 1) * 128]
            rr[rows, :] = _rb(jnp.sum(n * wr, axis=-1, keepdims=True))
            return 0
        lax.fori_loop(0, T // 32, ln, 0)
        for j in range(0, J, 2):
            for g in range(G):
                a = xn[g, pl.ds(i * T + j, 8, stride=J), :]
                b = xn[g, pl.ds(i * T + j + 1, 8, stride=J), :]
                xp[pl.ds(i * T + j * 8, 16), pl.ds(g * 128, 128)] = (
                    jnp.concatenate([a, b], axis=0).astype(bf16))

    r = rr[...]
    ti = lax.broadcasted_iota(jnp.int32, (L, 1), 0)
    m0 = jnp.max(r, axis=0, keepdims=True)
    i0v = jnp.min(jnp.where(r == m0, ti, L), axis=0, keepdims=True)
    r2 = jnp.where(ti == i0v, -jnp.inf, r)
    m1 = jnp.max(r2, axis=0, keepdims=True)
    i1v = jnp.min(jnp.where((r2 == m1) & (ti != i0v), ti, L), axis=0, keepdims=True)
    i0 = jnp.clip(i0v[0, 0], 0, L - 1)
    i1 = jnp.clip(i1v[0, 0], 0, L - 1)

    for c in b_cp + c_cp:
        c.wait()
    for q in range(D // 128):
        rows = pl.ds(q * 128, 128)
        cr, ci = cw[0, rows, :].astype(f32), cw[1, rows, :].astype(f32)
        cw[0, rows, :] = (2.0 * (cr * cfr - ci * cfi)).astype(bf16)
        cw[1, rows, :] = (-2.0 * (cr * cfi + ci * cfr)).astype(bf16)

    def mm1(i, bu):
        xx = xp[pl.ds(pl.multiple_of(i * T, T), T), :]
        bu[0] = lax.dot_general(xx, bw[0], NT, preferred_element_type=f32)
        bu[1] = lax.dot_general(xx, bw[1], NT, preferred_element_type=f32)

    def scan(bu, h):
        for g in range(G):
            ln_ = pl.ds(g * 128, 128)
            a_r, a_i = st[0, :, ln_], st[1, :, ln_]
            c_r, c_i = st[8, :, ln_], st[9, :, ln_]
            sr, si = c_r, c_i
            for j in range(J):
                rows = pl.ds(j * 8, 8)
                sr, si = (a_r * sr - a_i * si + bu[0, rows, ln_],
                          a_r * si + a_i * sr + bu[1, rows, ln_])
            for k in range(3):
                pr, pi = st[2 + 2 * k, :, ln_], st[3 + 2 * k, :, ln_]
                qr, qi = pltpu.roll(sr, 1 << k, 0), pltpu.roll(si, 1 << k, 0)
                sr, si = sr + (pr * qr - pi * qi), si + (pr * qi + pi * qr)
            er, ei = pltpu.roll(sr, 1, 0), pltpu.roll(si, 1, 0)
            first = lax.broadcasted_iota(jnp.int32, (8, 128), 0) == 0
            st[8, :, ln_] = jnp.where(first, er, 0.0)
            st[9, :, ln_] = jnp.where(first, ei, 0.0)
            sr, si = jnp.where(first, c_r, er), jnp.where(first, c_i, ei)
            for j in range(0, J, 2):
                o = []
                for jj in (j, j + 1):
                    rows = pl.ds(jj * 8, 8)
                    sr, si = (a_r * sr - a_i * si + bu[0, rows, ln_],
                              a_r * si + a_i * sr + bu[1, rows, ln_])
                    o.append((sr, si))
                rows = pl.ds(j * 8, 16)
                h[0, rows, ln_] = jnp.concatenate([o[0][0], o[1][0]], 0).astype(bf16)
                h[1, rows, ln_] = jnp.concatenate([o[0][1], o[1][1]], 0).astype(bf16)

    def mm2(i, h):
        y = (lax.dot_general(h[0], cw[0], NT, preferred_element_type=f32)
             + lax.dot_general(h[1], cw[1], NT, preferred_element_type=f32))
        for j in range(J):
            rows = pl.ds(i * T + j, 8, stride=J)
            for g in range(G):
                ob[g, rows, :] = ob[g, rows, :] + y[j * 8:(j + 1) * 8, g * 128:(g + 1) * 128]

    def out_cp(g):
        return pltpu.make_async_copy(ob.at[g], o_hbm.at[:, pl.ds(g * 128, 128)], osem.at[g])

    def get_row(ref, idx):
        return jnp.concatenate([ref[g, pl.ds(idx, 1), :] for g in range(G)], axis=1)

    mm1(0, bu0)
    mm1(1, bu1)
    scan(bu0, h0)

    def body(k, _):
        i = 2 * k
        mm2(i, h0)
        scan(bu1, h1)
        mm1(i + 2, bu0)
        mm2(i + 1, h1)
        scan(bu0, h0)
        mm1(i + 3, bu1)
        return 0
    lax.fori_loop(0, NB // 2 - 1, body, 0)
    mm2(NB - 2, h0)
    scan(bu1, h1)
    mm2(NB - 1, h1)

    for c in w_cp:
        c.wait()
    s8 = lax.broadcasted_iota(jnp.int32, (16, D), 0)
    xs = jnp.where(s8 == 0, get_row(xn, i0), jnp.where(s8 == 1, get_row(xn, i1), 0.0)).astype(bf16)
    acc = jnp.zeros((16, D), f32)
    for c in range(NF):
        cols = pl.ds(c * FC, FC)
        gt = _rb(jnp.dot(xs, wg[:, cols], preferred_element_type=f32))
        gt = _rb(gt * _rb(jax.nn.sigmoid(gt)))
        up = _rb(jnp.dot(xs, wu[:, cols], preferred_element_type=f32))
        acc = acc + jnp.dot((gt * up).astype(bf16), wd[cols, :], preferred_element_type=f32)
    yf = _rb(acc)
    for k, (idx, m) in enumerate(((i0, m0), (i1, m1))):
        row = pl.ds(idx, 1)
        n = get_row(xn, idx)
        upd = _rb(yf[k:k + 1, :] * _rb(jax.nn.sigmoid(m)))
        dl = _rb(n + upd) - n
        for g in range(G):
            ob[g, row, :] = ob[g, row, :] + dl[:, g * 128:(g + 1) * 128]
    for i in range(NB):
        out_cp(i).start()
    for i in range(NB):
        out_cp(i).wait()


@jax.jit
def pallas_parallel_sum__ssm_conv_s5__moe_arch_mod__prompt_kernel(
    A_x, A_Lambda_re, A_Lambda_im, A_B_re, A_B_im, A_C_re, A_C_im, A_log_dt, A_Dskip,
    B_x, B_w_r, B_w_gate, B_w_up, B_w_down,
):
    hbm = pl.BlockSpec(memory_space=pl.ANY)
    vm = pl.BlockSpec(memory_space=pltpu.VMEM)
    row = lambda v: v.reshape(1, -1)
    out = pl.pallas_call(
        _kernel,
        out_shape=jax.ShapeDtypeStruct((L, D), f32),
        in_specs=[hbm, vm, vm, hbm, hbm, hbm, hbm, vm, vm, vm, hbm, hbm, hbm],
        out_specs=hbm,
        scratch_shapes=[
            pltpu.VMEM((L, D), bf16), pltpu.VMEM((G, L, 128), f32), pltpu.VMEM((L, D), bf16),
            pltpu.VMEM((G, L, 128), f32),
            pltpu.VMEM((2, P, D), bf16), pltpu.VMEM((2, D, P), bf16),
            pltpu.VMEM((D, F), bf16), pltpu.VMEM((D, F), bf16), pltpu.VMEM((F, D), bf16),
            pltpu.VMEM((2, T, P), f32), pltpu.VMEM((2, T, P), f32),
            pltpu.VMEM((2, T, P), bf16), pltpu.VMEM((2, T, P), bf16),
            pltpu.VMEM((L, 1), f32), pltpu.VMEM((10, 8, P), f32),
            pltpu.SemaphoreType.DMA((NB + 7,)), pltpu.SemaphoreType.DMA((NB,)),
        ],
        compiler_params=pltpu.CompilerParams(vmem_limit_bytes=110 * 1024 * 1024),
    )(A_x.reshape(L, D), row(A_Lambda_re), row(A_Lambda_im), A_B_re, A_B_im, A_C_re, A_C_im,
      row(A_log_dt), row(A_Dskip), row(B_w_r), B_w_gate, B_w_up, B_w_down)
    return out.reshape(1, L, D)
```

```python
import jax
import jax.numpy as jnp
from jax import lax
import jax.experimental.pallas as pl
import jax.experimental.pallas.tpu as pltpu

L, D, P, F = 2048, 1024, 1024, 3584
T = 256
J = T // 8
NB = L // T
JP = J + 1
TP = 8 * JP
G = P // 128
FC = 512
NF = F // FC
f32, bf16 = jnp.float32, jnp.bfloat16
NT = (((1,), (1,)), ((), ()))


def _rb(v):
    return v.astype(bf16).astype(f32)


def _kernel(x_hbm, lre_ref, lim_ref, bre_hbm, bim_hbm, cre_hbm, cim_hbm, ldt_ref, dsk_ref,
            wr_ref, wg_hbm, wu_hbm, wd_hbm, o_hbm,
            xb, xn, xp0, xp1, ob, yb, bw, cw, wg, wu, wd, bu0, bu1, h0, h1, rr, st, sem, osem):
    def cp(src, dst, k):
        return pltpu.make_async_copy(src, dst, sem.at[k])

    x_cp = [cp(x_hbm.at[pl.ds(i * T, T)], xb.at[pl.ds(i * T, T)], i) for i in range(NB)]
    b_cp = [cp(bre_hbm, bw.at[0], NB), cp(bim_hbm, bw.at[1], NB + 1)]
    c_cp = [cp(cre_hbm, cw.at[0], NB + 2), cp(cim_hbm, cw.at[1], NB + 3)]
    w_cp = [cp(wg_hbm, wg, NB + 4), cp(wu_hbm, wu, NB + 5), cp(wd_hbm, wd, NB + 6)]
    for c in x_cp[:1] + b_cp + x_cp[1:3]:
        c.start()

    lre = lre_ref[...].astype(f32)
    lim = lim_ref[...].astype(f32)
    dt = _rb(jnp.exp(ldt_ref[...].astype(f32)))
    ar, ai = dt * lre, dt * lim
    mag = jnp.exp(ar)
    lbr, lbi = mag * jnp.cos(ai), mag * jnp.sin(ai)
    den = lre * lre + lim * lim
    cfr = ((lbr - 1.0) * lre + lbi * lim) / den
    cfi = (lbi * lre - (lbr - 1.0) * lim) / den
    st[0] = jnp.broadcast_to(lbr, (8, P))
    st[1] = jnp.broadcast_to(lbi, (8, P))
    sub = lax.broadcasted_iota(jnp.int32, (8, P), 0)
    for k in range(3):
        n = float(J * (1 << k))
        m = jnp.exp(ar * n)
        keep = sub >= (1 << k)
        st[2 + 2 * k] = jnp.where(keep, jnp.broadcast_to(m * jnp.cos(ai * n), (8, P)), 0.0)
        st[3 + 2 * k] = jnp.where(keep, jnp.broadcast_to(m * jnp.sin(ai * n), (8, P)), 0.0)
    st[8] = jnp.zeros((8, P), f32)
    st[9] = jnp.zeros((8, P), f32)

    dsk = dsk_ref[...].astype(f32)
    wr = wr_ref[...].astype(f32)

    def lnorm(i, xp):
        for q in range(8):
            rows = pl.ds(i * T + q * J, J)
            x = xb[rows, :].astype(f32)
            mu = jnp.mean(x, axis=-1, keepdims=True)
            c = x - mu
            var = _rb(jnp.mean(c * c, axis=-1, keepdims=True))
            s = _rb(jnp.sqrt(_rb(var + 1e-5)))
            n = _rb(_rb(x - _rb(mu)) * (1.0 / s))
            base = x + _rb(n * dsk) + n
            for g in range(G):
                xn[g, pl.ds(i * TP + q * JP, J), :] = n[:, g * 128:(g + 1) * 128]
            ob[rows, :] = base
            rr[rows, :] = _rb(jnp.sum(n * wr, axis=-1, keepdims=True))
        for j in range(0, J, 2):
            for g in range(G):
                a = xn[g, pl.ds(i * TP + j, 8, stride=JP), :]
                b = xn[g, pl.ds(i * TP + j + 1, 8, stride=JP), :]
                xp[pl.ds(j * 8, 16), pl.ds(g * 128, 128)] = (
                    jnp.concatenate([a, b], axis=0).astype(bf16))

    def x_wait(i):
        rows = pl.ds(i * T, T)
        pltpu.make_async_copy(x_hbm.at[rows], xb.at[rows], sem.at[i]).wait()

    def cfold():
        for q in range(D // 128):
            rows = pl.ds(q * 128, 128)
            cr, ci = cw[0, rows, :].astype(f32), cw[1, rows, :].astype(f32)
            cw[0, rows, :] = (2.0 * (cr * cfr - ci * cfi)).astype(bf16)
            cw[1, rows, :] = (-2.0 * (cr * cfi + ci * cfr)).astype(bf16)

    def mm1(xp, bu):
        xx = xp[...]
        bu[0] = lax.dot_general(xx, bw[0], NT, preferred_element_type=f32)
        bu[1] = lax.dot_general(xx, bw[1], NT, preferred_element_type=f32)

    def scan(bu, h):
        for g in range(G):
            ln_ = pl.ds(g * 128, 128)
            a_r, a_i = st[0, :, ln_], st[1, :, ln_]
            c_r, c_i = st[8, :, ln_], st[9, :, ln_]
            sr, si = c_r, c_i
            for j in range(J):
                rows = pl.ds(j * 8, 8)
                sr, si = (a_r * sr - a_i * si + bu[0, rows, ln_],
                          a_r * si + a_i * sr + bu[1, rows, ln_])
            for k in range(3):
                pr, pi = st[2 + 2 * k, :, ln_], st[3 + 2 * k, :, ln_]
                qr, qi = pltpu.roll(sr, 1 << k, 0), pltpu.roll(si, 1 << k, 0)
                sr, si = sr + (pr * qr - pi * qi), si + (pr * qi + pi * qr)
            er, ei = pltpu.roll(sr, 1, 0), pltpu.roll(si, 1, 0)
            first = lax.broadcasted_iota(jnp.int32, (8, 128), 0) == 0
            st[8, :, ln_] = jnp.where(first, er, 0.0)
            st[9, :, ln_] = jnp.where(first, ei, 0.0)
            sr, si = jnp.where(first, c_r, er), jnp.where(first, c_i, ei)
            for j in range(0, J, 2):
                o = []
                for jj in (j, j + 1):
                    rows = pl.ds(jj * 8, 8)
                    sr, si = (a_r * sr - a_i * si + bu[0, rows, ln_],
                              a_r * si + a_i * sr + bu[1, rows, ln_])
                    o.append((sr, si))
                rows = pl.ds(j * 8, 16)
                h[0, rows, ln_] = jnp.concatenate([o[0][0], o[1][0]], 0).astype(bf16)
                h[1, rows, ln_] = jnp.concatenate([o[0][1], o[1][1]], 0).astype(bf16)

    def mm2(i, h):
        y = (lax.dot_general(h[0], cw[0], NT, preferred_element_type=f32)
             + lax.dot_general(h[1], cw[1], NT, preferred_element_type=f32))
        for j in range(J):
            for g in range(G):
                yb[g, pl.ds(j, 8, stride=JP), :] = y[j * 8:(j + 1) * 8, g * 128:(g + 1) * 128]
        for q in range(8):
            rows = pl.ds(i * T + q * J, J)
            for g in range(G):
                cols = pl.ds(g * 128, 128)
                ob[rows, cols] = ob[rows, cols] + yb[g, pl.ds(q * JP, J), :]

    def out_cps(i):
        rows = pl.ds(i * T, T)
        return [pltpu.make_async_copy(ob.at[rows], o_hbm.at[rows], osem.at[i])]

    def get_row(ref, idx):
        return jnp.concatenate([ref[g, pl.ds(idx + idx // J, 1), :] for g in range(G)], axis=1)

    x_wait(0)
    lnorm(0, xp0)
    for c in b_cp:
        c.wait()
    for c in c_cp + x_cp[3:] + w_cp:
        c.start()
    x_wait(1)
    lnorm(1, xp1)
    mm1(xp0, bu0)
    x_wait(2)
    for c in c_cp:
        c.wait()
    cfold()
    lnorm(2, xp0)
    mm1(xp1, bu1)
    scan(bu0, h0)

    def body(k, _):
        i = 2 * k
        x_wait(i + 3)
        lnorm(i + 3, xp1)
        mm2(i, h0)
        scan(bu1, h1)
        mm1(xp0, bu0)
        x_wait(i + 4)
        lnorm(i + 4, xp0)
        mm2(i + 1, h1)
        scan(bu0, h0)
        mm1(xp1, bu1)
        return 0
    for k in range(NB // 2 - 2):
        body(k, 0)
    x_wait(NB - 1)
    lnorm(NB - 1, xp1)
    mm2(NB - 4, h0)
    scan(bu1, h1)
    mm1(xp0, bu0)
    r = rr[...]
    ti = lax.broadcasted_iota(jnp.int32, (L, 1), 0)
    m0 = jnp.max(r, axis=0, keepdims=True)
    i0v = jnp.min(jnp.where(r == m0, ti, L), axis=0, keepdims=True)
    r2 = jnp.where(ti == i0v, -jnp.inf, r)
    m1 = jnp.max(r2, axis=0, keepdims=True)
    i1v = jnp.min(jnp.where((r2 == m1) & (ti != i0v), ti, L), axis=0, keepdims=True)
    i0 = jnp.clip(i0v[0, 0], 0, L - 1)
    i1 = jnp.clip(i1v[0, 0], 0, L - 1)

    mm2(NB - 3, h1)
    scan(bu0, h0)
    mm1(xp1, bu1)

    for c in w_cp:
        c.wait()
    s8 = lax.broadcasted_iota(jnp.int32, (16, D), 0)
    xs = jnp.where(s8 == 0, get_row(xn, i0), jnp.where(s8 == 1, get_row(xn, i1), 0.0)).astype(bf16)
    acc = jnp.zeros((16, D), f32)
    for c in range(NF):
        cols = pl.ds(c * FC, FC)
        gt = _rb(jnp.dot(xs, wg[:, cols], preferred_element_type=f32))
        gt = _rb(gt * _rb(jax.nn.sigmoid(gt)))
        up = _rb(jnp.dot(xs, wu[:, cols], preferred_element_type=f32))
        acc = acc + jnp.dot((gt * up).astype(bf16), wd[cols, :], preferred_element_type=f32)
    yf = _rb(acc)
    for k, (idx, m) in enumerate(((i0, m0), (i1, m1))):
        row = pl.ds(idx, 1)
        n = get_row(xn, idx)
        upd = _rb(yf[k:k + 1, :] * _rb(jax.nn.sigmoid(m)))
        dl = _rb(n + upd) - n
        ob[row, :] = ob[row, :] + dl
    for i in range(NB - 2):
        for c in out_cps(i):
            c.start()
    mm2(NB - 2, h0)
    scan(bu1, h1)
    for c in out_cps(NB - 2):
        c.start()
    mm2(NB - 1, h1)
    for c in out_cps(NB - 1):
        c.start()
    for i in range(NB):
        for c in out_cps(i):
            c.wait()


@jax.jit
def pallas_parallel_sum__ssm_conv_s5__moe_arch_mod__prompt_kernel(
    A_x, A_Lambda_re, A_Lambda_im, A_B_re, A_B_im, A_C_re, A_C_im, A_log_dt, A_Dskip,
    B_x, B_w_r, B_w_gate, B_w_up, B_w_down,
):
    hbm = pl.BlockSpec(memory_space=pl.ANY)
    vm = pl.BlockSpec(memory_space=pltpu.VMEM)
    row = lambda v: v.reshape(1, -1)
    out = pl.pallas_call(
        _kernel,
        out_shape=jax.ShapeDtypeStruct((L, D), f32),
        in_specs=[hbm, vm, vm, hbm, hbm, hbm, hbm, vm, vm, vm, hbm, hbm, hbm],
        out_specs=hbm,
        scratch_shapes=[
            pltpu.VMEM((L, D), bf16), pltpu.VMEM((G, NB * TP, 128), f32), pltpu.VMEM((T, D), bf16),
            pltpu.VMEM((T, D), bf16), pltpu.VMEM((L, D), f32),
            pltpu.VMEM((G, TP, 128), f32),
            pltpu.VMEM((2, P, D), bf16), pltpu.VMEM((2, D, P), bf16),
            pltpu.VMEM((D, F), bf16), pltpu.VMEM((D, F), bf16), pltpu.VMEM((F, D), bf16),
            pltpu.VMEM((2, T, P), f32), pltpu.VMEM((2, T, P), f32),
            pltpu.VMEM((2, T, P), bf16), pltpu.VMEM((2, T, P), bf16),
            pltpu.VMEM((L, 1), f32), pltpu.VMEM((10, 8, P), f32),
            pltpu.SemaphoreType.DMA((NB + 7,)), pltpu.SemaphoreType.DMA((NB,)),
        ],
        compiler_params=pltpu.CompilerParams(vmem_limit_bytes=110 * 1024 * 1024),
    )(A_x.reshape(L, D), row(A_Lambda_re), row(A_Lambda_im), A_B_re, A_B_im, A_C_re, A_C_im,
      row(A_log_dt), row(A_Dskip), row(B_w_r), B_w_gate, B_w_up, B_w_down)
    return out.reshape(1, L, D)
```

```python
import jax
import jax.numpy as jnp
from jax import lax
import jax.experimental.pallas as pl
import jax.experimental.pallas.tpu as pltpu

L, D, P, F = 2048, 1024, 1024, 3584
T = 256
J = T // 8
NB = L // T
JP = J + 1
TP = 8 * JP
G = P // 128
FC = 512
NF = F // FC
f32, bf16 = jnp.float32, jnp.bfloat16
NT = (((1,), (1,)), ((), ()))


def _rb(v):
    return v.astype(bf16).astype(f32)


def _kernel(x_hbm, lre_ref, lim_ref, bre_hbm, bim_hbm, cre_hbm, cim_hbm, ldt_ref, dsk_ref,
            wr_ref, wg_hbm, wu_hbm, wd_hbm, o_hbm,
            xb, xn, xp0, xp1, ob, yb, bw, cw, wg, wu, wd, bu0, bu1, h0, h1, rr, st, sem, osem):
    def cp(src, dst, k):
        return pltpu.make_async_copy(src, dst, sem.at[k])

    x_cp = [cp(x_hbm.at[pl.ds(i * T, T)], xb.at[pl.ds(i * T, T)], i) for i in range(NB)]
    b_cp = [cp(bre_hbm, bw.at[0], NB), cp(bim_hbm, bw.at[1], NB + 1)]
    c_cp = [cp(cre_hbm, cw.at[0], NB + 2), cp(cim_hbm, cw.at[1], NB + 3)]
    w_cp = [cp(wg_hbm, wg, NB + 4), cp(wu_hbm, wu, NB + 5), cp(wd_hbm, wd, NB + 6)]
    for c in x_cp[:1] + b_cp[:1]:
        c.start()

    lre = lre_ref[...].astype(f32)
    lim = lim_ref[...].astype(f32)
    dt = _rb(jnp.exp(ldt_ref[...].astype(f32)))
    ar, ai = dt * lre, dt * lim
    mag = jnp.exp(ar)
    lbr, lbi = mag * jnp.cos(ai), mag * jnp.sin(ai)
    den = lre * lre + lim * lim
    cfr = ((lbr - 1.0) * lre + lbi * lim) / den
    cfi = (lbi * lre - (lbr - 1.0) * lim) / den
    st[0] = jnp.broadcast_to(lbr, (8, P))
    st[1] = jnp.broadcast_to(lbi, (8, P))
    sub = lax.broadcasted_iota(jnp.int32, (8, P), 0)
    for k in range(3):
        n = float(J * (1 << k))
        m = jnp.exp(ar * n)
        keep = sub >= (1 << k)
        st[2 + 2 * k] = jnp.where(keep, jnp.broadcast_to(m * jnp.cos(ai * n), (8, P)), 0.0)
        st[3 + 2 * k] = jnp.where(keep, jnp.broadcast_to(m * jnp.sin(ai * n), (8, P)), 0.0)
    st[8] = jnp.zeros((8, P), f32)
    st[9] = jnp.zeros((8, P), f32)

    dsk = dsk_ref[...].astype(f32)
    wr = wr_ref[...].astype(f32)

    def lnorm(i, xp):
        for q in range(8):
            rows = pl.ds(i * T + q * J, J)
            x = xb[rows, :].astype(f32)
            mu = jnp.mean(x, axis=-1, keepdims=True)
            c = x - mu
            var = _rb(jnp.mean(c * c, axis=-1, keepdims=True))
            s = _rb(jnp.sqrt(_rb(var + 1e-5)))
            n = _rb(_rb(x - _rb(mu)) * (1.0 / s))
            base = x + _rb(n * dsk) + n
            for g in range(G):
                xn[g, pl.ds(i * TP + q * JP, J), :] = n[:, g * 128:(g + 1) * 128]
            ob[rows, :] = base
            rr[rows, :] = _rb(jnp.sum(n * wr, axis=-1, keepdims=True))
        for j in range(0, J, 2):
            for g in range(G):
                a = xn[g, pl.ds(i * TP + j, 8, stride=JP), :]
                b = xn[g, pl.ds(i * TP + j + 1, 8, stride=JP), :]
                xp[pl.ds(j * 8, 16), pl.ds(g * 128, 128)] = (
                    jnp.concatenate([a, b], axis=0).astype(bf16))

    def x_wait(i):
        rows = pl.ds(i * T, T)
        pltpu.make_async_copy(x_hbm.at[rows], xb.at[rows], sem.at[i]).wait()

    def cfold():
        for q in range(D // 128):
            rows = pl.ds(q * 128, 128)
            cr, ci = cw[0, rows, :].astype(f32), cw[1, rows, :].astype(f32)
            cw[0, rows, :] = (2.0 * (cr * cfr - ci * cfi)).astype(bf16)
            cw[1, rows, :] = (-2.0 * (cr * cfi + ci * cfr)).astype(bf16)

    def mm1(xp, bu):
        xx = xp[...]
        bu[0] = lax.dot_general(xx, bw[0], NT, preferred_element_type=f32)
        bu[1] = lax.dot_general(xx, bw[1], NT, preferred_element_type=f32)

    def scan(bu, h):
        for g in range(G):
            ln_ = pl.ds(g * 128, 128)
            a_r, a_i = st[0, :, ln_], st[1, :, ln_]
            c_r, c_i = st[8, :, ln_], st[9, :, ln_]
            sr, si = c_r, c_i
            for j in range(J):
                rows = pl.ds(j * 8, 8)
                sr, si = (a_r * sr - a_i * si + bu[0, rows, ln_],
                          a_r * si + a_i * sr + bu[1, rows, ln_])
            for k in range(3):
                pr, pi = st[2 + 2 * k, :, ln_], st[3 + 2 * k, :, ln_]
                qr, qi = pltpu.roll(sr, 1 << k, 0), pltpu.roll(si, 1 << k, 0)
                sr, si = sr + (pr * qr - pi * qi), si + (pr * qi + pi * qr)
            er, ei = pltpu.roll(sr, 1, 0), pltpu.roll(si, 1, 0)
            first = lax.broadcasted_iota(jnp.int32, (8, 128), 0) == 0
            st[8, :, ln_] = jnp.where(first, er, 0.0)
            st[9, :, ln_] = jnp.where(first, ei, 0.0)
            sr, si = jnp.where(first, c_r, er), jnp.where(first, c_i, ei)
            for j in range(0, J, 2):
                o = []
                for jj in (j, j + 1):
                    rows = pl.ds(jj * 8, 8)
                    sr, si = (a_r * sr - a_i * si + bu[0, rows, ln_],
                              a_r * si + a_i * sr + bu[1, rows, ln_])
                    o.append((sr, si))
                rows = pl.ds(j * 8, 16)
                h[0, rows, ln_] = jnp.concatenate([o[0][0], o[1][0]], 0).astype(bf16)
                h[1, rows, ln_] = jnp.concatenate([o[0][1], o[1][1]], 0).astype(bf16)

    def mm2(i, h, g0=0, g1=G):
        wrows = pl.ds(g0 * 128, (g1 - g0) * 128)
        y = (lax.dot_general(h[0], cw[0, wrows, :], NT, preferred_element_type=f32)
             + lax.dot_general(h[1], cw[1, wrows, :], NT, preferred_element_type=f32))
        for j in range(J):
            for g in range(g0, g1):
                yb[g, pl.ds(j, 8, stride=JP), :] = (
                    y[j * 8:(j + 1) * 8, (g - g0) * 128:(g - g0 + 1) * 128])
        for q in range(8):
            rows = pl.ds(i * T + q * J, J)
            for g in range(g0, g1):
                cols = pl.ds(g * 128, 128)
                ob[rows, cols] = ob[rows, cols] + yb[g, pl.ds(q * JP, J), :]

    def last_cp(q):
        rows, cols = pl.ds((NB - 1) * T, T), pl.ds(q * 512, 512)
        return pltpu.make_async_copy(ob.at[rows, cols], o_hbm.at[rows, cols], osem.at[NB - 1 + q])

    def out_cps(i):
        rows = pl.ds(i * T, T)
        return [pltpu.make_async_copy(ob.at[rows], o_hbm.at[rows], osem.at[i])]

    def get_row(ref, idx):
        return jnp.concatenate([ref[g, pl.ds(idx + idx // J, 1), :] for g in range(G)], axis=1)

    x_wait(0)
    for c in b_cp[1:] + x_cp[1:3]:
        c.start()
    lnorm(0, xp0)
    b_cp[0].wait()
    for c in c_cp:
        c.start()
    bu0[0] = lax.dot_general(xp0[...], bw[0], NT, preferred_element_type=f32)
    b_cp[1].wait()
    x_wait(1)
    for c in x_cp[3:]:
        c.start()
    lnorm(1, xp1)
    bu0[1] = lax.dot_general(xp0[...], bw[1], NT, preferred_element_type=f32)
    x_wait(2)
    for c in w_cp:
        c.start()
    for c in c_cp:
        c.wait()
    cfold()
    lnorm(2, xp0)
    mm1(xp1, bu1)
    scan(bu0, h0)

    def body(k, _):
        i = 2 * k
        x_wait(i + 3)
        lnorm(i + 3, xp1)
        mm2(i, h0)
        scan(bu1, h1)
        mm1(xp0, bu0)
        x_wait(i + 4)
        lnorm(i + 4, xp0)
        mm2(i + 1, h1)
        scan(bu0, h0)
        mm1(xp1, bu1)
        return 0
    for k in range(NB // 2 - 2):
        body(k, 0)
    x_wait(NB - 1)
    lnorm(NB - 1, xp1)
    mm2(NB - 4, h0)
    scan(bu1, h1)
    mm1(xp0, bu0)
    r = rr[...]
    ti = lax.broadcasted_iota(jnp.int32, (L, 1), 0)
    m0 = jnp.max(r, axis=0, keepdims=True)
    i0v = jnp.min(jnp.where(r == m0, ti, L), axis=0, keepdims=True)
    r2 = jnp.where(ti == i0v, -jnp.inf, r)
    m1 = jnp.max(r2, axis=0, keepdims=True)
    i1v = jnp.min(jnp.where((r2 == m1) & (ti != i0v), ti, L), axis=0, keepdims=True)
    i0 = jnp.clip(i0v[0, 0], 0, L - 1)
    i1 = jnp.clip(i1v[0, 0], 0, L - 1)

    for c in w_cp:
        c.wait()
    mm2(NB - 3, h1)
    scan(bu0, h0)
    mm1(xp1, bu1)
    s8 = lax.broadcasted_iota(jnp.int32, (16, D), 0)
    xs = jnp.where(s8 == 0, get_row(xn, i0), jnp.where(s8 == 1, get_row(xn, i1), 0.0)).astype(bf16)
    acc = jnp.zeros((16, D), f32)
    for c in range(NF):
        cols = pl.ds(c * FC, FC)
        gt = _rb(jnp.dot(xs, wg[:, cols], preferred_element_type=f32))
        gt = _rb(gt * _rb(jax.nn.sigmoid(gt)))
        up = _rb(jnp.dot(xs, wu[:, cols], preferred_element_type=f32))
        acc = acc + jnp.dot((gt * up).astype(bf16), wd[cols, :], preferred_element_type=f32)
    yf = _rb(acc)
    for k, (idx, m) in enumerate(((i0, m0), (i1, m1))):
        row = pl.ds(idx, 1)
        n = get_row(xn, idx)
        upd = _rb(yf[k:k + 1, :] * _rb(jax.nn.sigmoid(m)))
        dl = _rb(n + upd) - n
        ob[row, :] = ob[row, :] + dl
    for i in range(NB - 2):
        for c in out_cps(i):
            c.start()
    mm2(NB - 2, h0)
    scan(bu1, h1)
    for c in out_cps(NB - 2):
        c.start()
    for q in range(2):
        mm2(NB - 1, h1, 4 * q, 4 * q + 4)
        last_cp(q).start()
    for i in range(NB - 1):
        for c in out_cps(i):
            c.wait()
    for q in range(2):
        last_cp(q).wait()


@jax.jit
def pallas_parallel_sum__ssm_conv_s5__moe_arch_mod__prompt_kernel(
    A_x, A_Lambda_re, A_Lambda_im, A_B_re, A_B_im, A_C_re, A_C_im, A_log_dt, A_Dskip,
    B_x, B_w_r, B_w_gate, B_w_up, B_w_down,
):
    hbm = pl.BlockSpec(memory_space=pl.ANY)
    vm = pl.BlockSpec(memory_space=pltpu.VMEM)
    row = lambda v: v.reshape(1, -1)
    out = pl.pallas_call(
        _kernel,
        out_shape=jax.ShapeDtypeStruct((L, D), f32),
        in_specs=[hbm, vm, vm, hbm, hbm, hbm, hbm, vm, vm, vm, hbm, hbm, hbm],
        out_specs=hbm,
        scratch_shapes=[
            pltpu.VMEM((L, D), bf16), pltpu.VMEM((G, NB * TP, 128), f32), pltpu.VMEM((T, D), bf16),
            pltpu.VMEM((T, D), bf16), pltpu.VMEM((L, D), f32),
            pltpu.VMEM((G, TP, 128), f32),
            pltpu.VMEM((2, P, D), bf16), pltpu.VMEM((2, D, P), bf16),
            pltpu.VMEM((D, F), bf16), pltpu.VMEM((D, F), bf16), pltpu.VMEM((F, D), bf16),
            pltpu.VMEM((2, T, P), f32), pltpu.VMEM((2, T, P), f32),
            pltpu.VMEM((2, T, P), bf16), pltpu.VMEM((2, T, P), bf16),
            pltpu.VMEM((L, 1), f32), pltpu.VMEM((10, 8, P), f32),
            pltpu.SemaphoreType.DMA((NB + 7,)), pltpu.SemaphoreType.DMA((NB + 1,)),
        ],
        compiler_params=pltpu.CompilerParams(vmem_limit_bytes=110 * 1024 * 1024),
    )(A_x.reshape(L, D), row(A_Lambda_re), row(A_Lambda_im), A_B_re, A_B_im, A_C_re, A_C_im,
      row(A_log_dt), row(A_Dskip), row(B_w_r), B_w_gate, B_w_up, B_w_down)
    return out.reshape(1, L, D)
```

```python
import jax
import jax.numpy as jnp
from jax import lax
import jax.experimental.pallas as pl
import jax.experimental.pallas.tpu as pltpu

L, D, P, F = 2048, 1024, 1024, 3584
T = 256
J = T // 8
NB = L // T
JP = J + 1
TP = 8 * JP
G = P // 128
FC = 512
NF = F // FC
f32, bf16 = jnp.float32, jnp.bfloat16
NT = (((1,), (1,)), ((), ()))


def _rb(v):
    return v.astype(bf16).astype(f32)


def _kernel(x_hbm, lre_ref, lim_ref, bre_hbm, bim_hbm, cre_hbm, cim_hbm, ldt_ref, dsk_ref,
            wr_ref, wg_hbm, wu_hbm, wd_hbm, o_hbm,
            xb, xn, xp0, xp1, ob, yb, bw, cw, wg, wu, wd, bu0, bu1, h0, h1, rr, st, sem, osem):
    def cp(src, dst, k):
        return pltpu.make_async_copy(src, dst, sem.at[k])

    x_cp = [cp(x_hbm.at[pl.ds(i * T, T)], xb.at[pl.ds(i * T, T)], i) for i in range(NB)]
    b_cp = [cp(bre_hbm, bw.at[0], NB), cp(bim_hbm, bw.at[1], NB + 1)]
    c_cp = [cp(cre_hbm, cw.at[0], NB + 2), cp(cim_hbm, cw.at[1], NB + 3)]
    w_cp = [cp(wg_hbm, wg, NB + 4), cp(wu_hbm, wu, NB + 5), cp(wd_hbm, wd, NB + 6)]
    for c in x_cp[:1] + b_cp[:1]:
        c.start()

    lre = lre_ref[...].astype(f32)
    lim = lim_ref[...].astype(f32)
    dt = _rb(jnp.exp(ldt_ref[...].astype(f32)))
    ar, ai = dt * lre, dt * lim
    mag = jnp.exp(ar)
    lbr, lbi = mag * jnp.cos(ai), mag * jnp.sin(ai)
    den = lre * lre + lim * lim
    cfr = ((lbr - 1.0) * lre + lbi * lim) / den
    cfi = (lbi * lre - (lbr - 1.0) * lim) / den
    st[0] = jnp.broadcast_to(lbr, (8, P))
    st[1] = jnp.broadcast_to(lbi, (8, P))
    sub = lax.broadcasted_iota(jnp.int32, (8, P), 0)
    for k in range(3):
        n = float(J * (1 << k))
        m = jnp.exp(ar * n)
        keep = sub >= (1 << k)
        st[2 + 2 * k] = jnp.where(keep, jnp.broadcast_to(m * jnp.cos(ai * n), (8, P)), 0.0)
        st[3 + 2 * k] = jnp.where(keep, jnp.broadcast_to(m * jnp.sin(ai * n), (8, P)), 0.0)
    st[10] = jnp.broadcast_to(2.0 * cfr, (8, P))
    st[11] = jnp.broadcast_to(2.0 * cfi, (8, P))
    st[8] = jnp.zeros((8, P), f32)
    st[9] = jnp.zeros((8, P), f32)

    dsk = dsk_ref[...].astype(f32)
    wr = wr_ref[...].astype(f32)

    def lnorm(i, xp):
        for q in range(8):
            rows = pl.ds(i * T + q * J, J)
            x = xb[rows, :].astype(f32)
            mu = jnp.mean(x, axis=-1, keepdims=True)
            c = x - mu
            var = _rb(jnp.mean(c * c, axis=-1, keepdims=True))
            s = _rb(jnp.sqrt(_rb(var + 1e-5)))
            n = _rb(_rb(x - _rb(mu)) * (1.0 / s))
            base = x + _rb(n * dsk) + n
            for g in range(G):
                xn[g, pl.ds(i * TP + q * JP, J), :] = n[:, g * 128:(g + 1) * 128]
            ob[rows, :] = base
            rr[rows, :] = _rb(jnp.sum(n * wr, axis=-1, keepdims=True))
        for j in range(0, J, 2):
            for g in range(G):
                a = xn[g, pl.ds(i * TP + j, 8, stride=JP), :]
                b = xn[g, pl.ds(i * TP + j + 1, 8, stride=JP), :]
                xp[pl.ds(j * 8, 16), pl.ds(g * 128, 128)] = (
                    jnp.concatenate([a, b], axis=0).astype(bf16))

    def x_wait(i):
        rows = pl.ds(i * T, T)
        pltpu.make_async_copy(x_hbm.at[rows], xb.at[rows], sem.at[i]).wait()

    def mm1(xp, bu):
        xx = xp[...]
        bu[0] = lax.dot_general(xx, bw[0], NT, preferred_element_type=f32)
        bu[1] = lax.dot_general(xx, bw[1], NT, preferred_element_type=f32)

    def scan(bu, h):
        for g in range(G):
            ln_ = pl.ds(g * 128, 128)
            a_r, a_i = st[0, :, ln_], st[1, :, ln_]
            k_r, k_i = st[10, :, ln_], st[11, :, ln_]
            c_r, c_i = st[8, :, ln_], st[9, :, ln_]
            sr, si = c_r, c_i
            for j in range(J):
                rows = pl.ds(j * 8, 8)
                sr, si = (a_r * sr - a_i * si + bu[0, rows, ln_],
                          a_r * si + a_i * sr + bu[1, rows, ln_])
            for k in range(3):
                pr, pi = st[2 + 2 * k, :, ln_], st[3 + 2 * k, :, ln_]
                qr, qi = pltpu.roll(sr, 1 << k, 0), pltpu.roll(si, 1 << k, 0)
                sr, si = sr + (pr * qr - pi * qi), si + (pr * qi + pi * qr)
            er, ei = pltpu.roll(sr, 1, 0), pltpu.roll(si, 1, 0)
            first = lax.broadcasted_iota(jnp.int32, (8, 128), 0) == 0
            st[8, :, ln_] = jnp.where(first, er, 0.0)
            st[9, :, ln_] = jnp.where(first, ei, 0.0)
            sr, si = jnp.where(first, c_r, er), jnp.where(first, c_i, ei)
            for j in range(0, J, 2):
                o = []
                for jj in (j, j + 1):
                    rows = pl.ds(jj * 8, 8)
                    sr, si = (a_r * sr - a_i * si + bu[0, rows, ln_],
                              a_r * si + a_i * sr + bu[1, rows, ln_])
                    o.append((sr * k_r - si * k_i, (-sr) * k_i - si * k_r))
                rows = pl.ds(j * 8, 16)
                h[0, rows, ln_] = jnp.concatenate([o[0][0], o[1][0]], 0).astype(bf16)
                h[1, rows, ln_] = jnp.concatenate([o[0][1], o[1][1]], 0).astype(bf16)

    def mm2(i, h, g0=0, g1=G):
        wrows = pl.ds(g0 * 128, (g1 - g0) * 128)
        y = (lax.dot_general(h[0], cw[0, wrows, :], NT, preferred_element_type=f32)
             + lax.dot_general(h[1], cw[1, wrows, :], NT, preferred_element_type=f32))
        for j in range(J):
            for g in range(g0, g1):
                yb[g, pl.ds(j, 8, stride=JP), :] = (
                    y[j * 8:(j + 1) * 8, (g - g0) * 128:(g - g0 + 1) * 128])
        for q in range(8):
            rows = pl.ds(i * T + q * J, J)
            for g in range(g0, g1):
                cols = pl.ds(g * 128, 128)
                ob[rows, cols] = ob[rows, cols] + yb[g, pl.ds(q * JP, J), :]

    def last_cp(q):
        rows, cols = pl.ds((NB - 1) * T, T), pl.ds(q * 512, 512)
        return pltpu.make_async_copy(ob.at[rows, cols], o_hbm.at[rows, cols], osem.at[NB - 1 + q])

    def out_cps(i):
        rows = pl.ds(i * T, T)
        return [pltpu.make_async_copy(ob.at[rows], o_hbm.at[rows], osem.at[i])]

    def get_row(ref, idx):
        return jnp.concatenate([ref[g, pl.ds(idx + idx // J, 1), :] for g in range(G)], axis=1)

    x_wait(0)
    for c in b_cp[1:] + x_cp[1:3]:
        c.start()
    lnorm(0, xp0)
    b_cp[0].wait()
    for c in c_cp:
        c.start()
    bu0[0] = lax.dot_general(xp0[...], bw[0], NT, preferred_element_type=f32)
    b_cp[1].wait()
    x_wait(1)
    for c in x_cp[3:]:
        c.start()
    lnorm(1, xp1)
    bu0[1] = lax.dot_general(xp0[...], bw[1], NT, preferred_element_type=f32)
    x_wait(2)
    for c in w_cp:
        c.start()
    for c in c_cp:
        c.wait()
    lnorm(2, xp0)
    mm1(xp1, bu1)
    scan(bu0, h0)

    def body(k, _):
        i = 2 * k
        x_wait(i + 3)
        lnorm(i + 3, xp1)
        mm2(i, h0)
        scan(bu1, h1)
        mm1(xp0, bu0)
        x_wait(i + 4)
        lnorm(i + 4, xp0)
        mm2(i + 1, h1)
        scan(bu0, h0)
        mm1(xp1, bu1)
        return 0
    for k in range(NB // 2 - 2):
        body(k, 0)
    x_wait(NB - 1)
    lnorm(NB - 1, xp1)
    mm2(NB - 4, h0)
    scan(bu1, h1)
    mm1(xp0, bu0)
    r = rr[...]
    ti = lax.broadcasted_iota(jnp.int32, (L, 1), 0)
    m0 = jnp.max(r, axis=0, keepdims=True)
    i0v = jnp.min(jnp.where(r == m0, ti, L), axis=0, keepdims=True)
    r2 = jnp.where(ti == i0v, -jnp.inf, r)
    m1 = jnp.max(r2, axis=0, keepdims=True)
    i1v = jnp.min(jnp.where((r2 == m1) & (ti != i0v), ti, L), axis=0, keepdims=True)
    i0 = jnp.clip(i0v[0, 0], 0, L - 1)
    i1 = jnp.clip(i1v[0, 0], 0, L - 1)

    for c in w_cp:
        c.wait()
    mm2(NB - 3, h1)
    scan(bu0, h0)
    mm1(xp1, bu1)
    s8 = lax.broadcasted_iota(jnp.int32, (16, D), 0)
    xs = jnp.where(s8 == 0, get_row(xn, i0), jnp.where(s8 == 1, get_row(xn, i1), 0.0)).astype(bf16)
    acc = jnp.zeros((16, D), f32)
    for c in range(NF):
        cols = pl.ds(c * FC, FC)
        gt = _rb(jnp.dot(xs, wg[:, cols], preferred_element_type=f32))
        gt = _rb(gt * _rb(jax.nn.sigmoid(gt)))
        up = _rb(jnp.dot(xs, wu[:, cols], preferred_element_type=f32))
        acc = acc + jnp.dot((gt * up).astype(bf16), wd[cols, :], preferred_element_type=f32)
    yf = _rb(acc)
    for k, (idx, m) in enumerate(((i0, m0), (i1, m1))):
        row = pl.ds(idx, 1)
        n = get_row(xn, idx)
        upd = _rb(yf[k:k + 1, :] * _rb(jax.nn.sigmoid(m)))
        dl = _rb(n + upd) - n
        ob[row, :] = ob[row, :] + dl
    for i in range(NB - 2):
        for c in out_cps(i):
            c.start()
    mm2(NB - 2, h0)
    scan(bu1, h1)
    for c in out_cps(NB - 2):
        c.start()
    for q in range(2):
        mm2(NB - 1, h1, 4 * q, 4 * q + 4)
        last_cp(q).start()
    for i in range(NB - 1):
        for c in out_cps(i):
            c.wait()
    for q in range(2):
        last_cp(q).wait()


@jax.jit
def pallas_parallel_sum__ssm_conv_s5__moe_arch_mod__prompt_kernel(
    A_x, A_Lambda_re, A_Lambda_im, A_B_re, A_B_im, A_C_re, A_C_im, A_log_dt, A_Dskip,
    B_x, B_w_r, B_w_gate, B_w_up, B_w_down,
):
    hbm = pl.BlockSpec(memory_space=pl.ANY)
    vm = pl.BlockSpec(memory_space=pltpu.VMEM)
    row = lambda v: v.reshape(1, -1)
    out = pl.pallas_call(
        _kernel,
        out_shape=jax.ShapeDtypeStruct((L, D), f32),
        in_specs=[hbm, vm, vm, hbm, hbm, hbm, hbm, vm, vm, vm, hbm, hbm, hbm],
        out_specs=hbm,
        scratch_shapes=[
            pltpu.VMEM((L, D), bf16), pltpu.VMEM((G, NB * TP, 128), f32), pltpu.VMEM((T, D), bf16),
            pltpu.VMEM((T, D), bf16), pltpu.VMEM((L, D), f32),
            pltpu.VMEM((G, TP, 128), f32),
            pltpu.VMEM((2, P, D), bf16), pltpu.VMEM((2, D, P), bf16),
            pltpu.VMEM((D, F), bf16), pltpu.VMEM((D, F), bf16), pltpu.VMEM((F, D), bf16),
            pltpu.VMEM((2, T, P), f32), pltpu.VMEM((2, T, P), f32),
            pltpu.VMEM((2, T, P), bf16), pltpu.VMEM((2, T, P), bf16),
            pltpu.VMEM((L, 1), f32), pltpu.VMEM((12, 8, P), f32),
            pltpu.SemaphoreType.DMA((NB + 7,)), pltpu.SemaphoreType.DMA((NB + 1,)),
        ],
        compiler_params=pltpu.CompilerParams(vmem_limit_bytes=110 * 1024 * 1024),
    )(A_x.reshape(L, D), row(A_Lambda_re), row(A_Lambda_im), A_B_re, A_B_im, A_C_re, A_C_im,
      row(A_log_dt), row(A_Dskip), row(B_w_r), B_w_gate, B_w_up, B_w_down)
    return out.reshape(1, L, D)
```

```python
import jax
import jax.numpy as jnp
from jax import lax
import jax.experimental.pallas as pl
import jax.experimental.pallas.tpu as pltpu

L, D, P, F = 2048, 1024, 1024, 3584
T = 256
J = T // 8
NB = L // T
JP = J + 1
TP = 8 * JP
G = P // 128
FC = 512
NF = F // FC
f32, bf16 = jnp.float32, jnp.bfloat16
NT = (((1,), (1,)), ((), ()))


def _rb(v):
    return v.astype(bf16).astype(f32)


def _kernel(x_hbm, lre_ref, lim_ref, bre_hbm, bim_hbm, cre_hbm, cim_hbm, ldt_ref, dsk_ref,
            wr_ref, wg_hbm, wu_hbm, wd_hbm, o_hbm,
            xb, xn, xp0, xp1, ob, yb, bw, cw, wg, wu, wd, bu0, bu1, h0, h1, rr, st, sem, osem):
    def cp(src, dst, k):
        return pltpu.make_async_copy(src, dst, sem.at[k])

    x_cp = [cp(x_hbm.at[pl.ds(i * T, T)], xb.at[pl.ds(i * T, T)], i) for i in range(NB)]
    b_cp = [cp(bre_hbm, bw.at[0], NB), cp(bim_hbm, bw.at[1], NB + 1)]
    c_cp = [cp(cre_hbm, cw.at[0], NB + 2), cp(cim_hbm, cw.at[1], NB + 3)]
    w_cp = [cp(wg_hbm, wg, NB + 4), cp(wu_hbm, wu, NB + 5), cp(wd_hbm, wd, NB + 6)]
    for c in x_cp[:1] + b_cp[:1]:
        c.start()

    lre = lre_ref[...].astype(f32)
    lim = lim_ref[...].astype(f32)
    dt = _rb(jnp.exp(ldt_ref[...].astype(f32)))
    ar, ai = dt * lre, dt * lim
    mag = jnp.exp(ar)
    lbr, lbi = mag * jnp.cos(ai), mag * jnp.sin(ai)
    den = lre * lre + lim * lim
    cfr = ((lbr - 1.0) * lre + lbi * lim) / den
    cfi = (lbi * lre - (lbr - 1.0) * lim) / den
    st[0] = jnp.broadcast_to(lbr, (8, P))
    st[1] = jnp.broadcast_to(lbi, (8, P))
    sub = lax.broadcasted_iota(jnp.int32, (8, P), 0)
    for k in range(3):
        n = float(J * (1 << k))
        m = jnp.exp(ar * n)
        keep = sub >= (1 << k)
        st[2 + 2 * k] = jnp.where(keep, jnp.broadcast_to(m * jnp.cos(ai * n), (8, P)), 0.0)
        st[3 + 2 * k] = jnp.where(keep, jnp.broadcast_to(m * jnp.sin(ai * n), (8, P)), 0.0)
    st[10] = jnp.broadcast_to(2.0 * cfr, (8, P))
    st[11] = jnp.broadcast_to(2.0 * cfi, (8, P))
    st[8] = jnp.zeros((8, P), f32)
    st[9] = jnp.zeros((8, P), f32)

    dsk = dsk_ref[...].astype(f32)
    wr = wr_ref[...].astype(f32)

    def lnorm(i, xp):
        for q in range(8):
            rows = pl.ds(i * T + q * J, J)
            x = xb[rows, :].astype(f32)
            mu = jnp.mean(x, axis=-1, keepdims=True)
            c = x - mu
            var = _rb(jnp.mean(c * c, axis=-1, keepdims=True))
            s = _rb(jnp.sqrt(_rb(var + 1e-5)))
            n = _rb(_rb(x - _rb(mu)) * (1.0 / s))
            base = x + _rb(n * dsk) + n
            for g in range(G):
                xn[g, pl.ds(i * TP + q * JP, J), :] = n[:, g * 128:(g + 1) * 128]
            ob[rows, :] = base
            rr[rows, :] = _rb(jnp.sum(n * wr, axis=-1, keepdims=True))
        for j in range(0, J, 2):
            for g in range(G):
                a = xn[g, pl.ds(i * TP + j, 8, stride=JP), :]
                b = xn[g, pl.ds(i * TP + j + 1, 8, stride=JP), :]
                xp[pl.ds(j * 8, 16), pl.ds(g * 128, 128)] = (
                    jnp.concatenate([a, b], axis=0).astype(bf16))

    def x_wait(i):
        rows = pl.ds(i * T, T)
        pltpu.make_async_copy(x_hbm.at[rows], xb.at[rows], sem.at[i]).wait()

    def mm1(xp, bu):
        xx = xp[...]
        bu[0] = lax.dot_general(xx, bw[0], NT, preferred_element_type=f32)
        bu[1] = lax.dot_general(xx, bw[1], NT, preferred_element_type=f32)

    def scan(bu, h):
        for g in range(G):
            ln_ = pl.ds(g * 128, 128)
            a_r, a_i = st[0, :, ln_], st[1, :, ln_]
            k_r, k_i = st[10, :, ln_], st[11, :, ln_]
            c_r, c_i = st[8, :, ln_], st[9, :, ln_]
            sr, si = c_r, c_i
            for j in range(J):
                rows = pl.ds(j * 8, 8)
                sr, si = (a_r * sr - a_i * si + bu[0, rows, ln_],
                          a_r * si + a_i * sr + bu[1, rows, ln_])
            for k in range(3):
                pr, pi = st[2 + 2 * k, :, ln_], st[3 + 2 * k, :, ln_]
                qr, qi = pltpu.roll(sr, 1 << k, 0), pltpu.roll(si, 1 << k, 0)
                sr, si = sr + (pr * qr - pi * qi), si + (pr * qi + pi * qr)
            er, ei = pltpu.roll(sr, 1, 0), pltpu.roll(si, 1, 0)
            first = lax.broadcasted_iota(jnp.int32, (8, 128), 0) == 0
            st[8, :, ln_] = jnp.where(first, er, 0.0)
            st[9, :, ln_] = jnp.where(first, ei, 0.0)
            sr, si = jnp.where(first, c_r, er), jnp.where(first, c_i, ei)
            for j in range(0, J, 2):
                o = []
                for jj in (j, j + 1):
                    rows = pl.ds(jj * 8, 8)
                    sr, si = (a_r * sr - a_i * si + bu[0, rows, ln_],
                              a_r * si + a_i * sr + bu[1, rows, ln_])
                    o.append((sr * k_r - si * k_i, (-sr) * k_i - si * k_r))
                rows = pl.ds(j * 8, 16)
                h[0, rows, ln_] = jnp.concatenate([o[0][0], o[1][0]], 0).astype(bf16)
                h[1, rows, ln_] = jnp.concatenate([o[0][1], o[1][1]], 0).astype(bf16)

    def mm2(i, h, g0=0, g1=G):
        wrows = pl.ds(g0 * 128, (g1 - g0) * 128)
        y = (lax.dot_general(h[0], cw[0, wrows, :], NT, preferred_element_type=f32)
             + lax.dot_general(h[1], cw[1, wrows, :], NT, preferred_element_type=f32))
        for j in range(J):
            for g in range(g0, g1):
                yb[g, pl.ds(j, 8, stride=JP), :] = (
                    y[j * 8:(j + 1) * 8, (g - g0) * 128:(g - g0 + 1) * 128])
        for q in range(8):
            rows = pl.ds(i * T + q * J, J)
            for g in range(g0, g1):
                cols = pl.ds(g * 128, 128)
                ob[rows, cols] = ob[rows, cols] + yb[g, pl.ds(q * JP, J), :]

    def last_cp(q):
        rows, cols = pl.ds((NB - 1) * T, T), pl.ds(q * 512, 512)
        return pltpu.make_async_copy(ob.at[rows, cols], o_hbm.at[rows, cols], osem.at[NB - 1 + q])

    def out_cps(i):
        rows = pl.ds(i * T, T)
        return [pltpu.make_async_copy(ob.at[rows], o_hbm.at[rows], osem.at[i])]

    def get_row(ref, idx):
        return jnp.concatenate([ref[g, pl.ds(idx + idx // J, 1), :] for g in range(G)], axis=1)

    x_wait(0)
    for c in b_cp[1:] + x_cp[1:2]:
        c.start()
    lnorm(0, xp0)
    b_cp[0].wait()
    x_cp[2].start()
    bu0[0] = lax.dot_general(xp0[...], bw[0], NT, preferred_element_type=f32)
    b_cp[1].wait()
    x_wait(1)
    for c in c_cp + x_cp[3:4]:
        c.start()
    lnorm(1, xp1)
    bu0[1] = lax.dot_general(xp0[...], bw[1], NT, preferred_element_type=f32)
    x_wait(2)
    lnorm(2, xp0)
    mm1(xp1, bu1)
    scan(bu0, h0)
    for c in c_cp:
        c.wait()
    for c in x_cp[4:] + w_cp:
        c.start()

    def body(k, _):
        i = 2 * k
        x_wait(i + 3)
        lnorm(i + 3, xp1)
        mm2(i, h0)
        scan(bu1, h1)
        mm1(xp0, bu0)
        x_wait(i + 4)
        lnorm(i + 4, xp0)
        mm2(i + 1, h1)
        scan(bu0, h0)
        mm1(xp1, bu1)
        return 0
    for k in range(NB // 2 - 2):
        body(k, 0)
    x_wait(NB - 1)
    lnorm(NB - 1, xp1)
    mm2(NB - 4, h0)
    scan(bu1, h1)
    mm1(xp0, bu0)
    r = rr[...]
    ti = lax.broadcasted_iota(jnp.int32, (L, 1), 0)
    m0 = jnp.max(r, axis=0, keepdims=True)
    i0v = jnp.min(jnp.where(r == m0, ti, L), axis=0, keepdims=True)
    r2 = jnp.where(ti == i0v, -jnp.inf, r)
    m1 = jnp.max(r2, axis=0, keepdims=True)
    i1v = jnp.min(jnp.where((r2 == m1) & (ti != i0v), ti, L), axis=0, keepdims=True)
    i0 = jnp.clip(i0v[0, 0], 0, L - 1)
    i1 = jnp.clip(i1v[0, 0], 0, L - 1)

    for c in w_cp:
        c.wait()
    mm2(NB - 3, h1)
    scan(bu0, h0)
    mm1(xp1, bu1)
    s8 = lax.broadcasted_iota(jnp.int32, (16, D), 0)
    xs = jnp.where(s8 == 0, get_row(xn, i0), jnp.where(s8 == 1, get_row(xn, i1), 0.0)).astype(bf16)
    acc = jnp.zeros((16, D), f32)
    for c in range(NF):
        cols = pl.ds(c * FC, FC)
        gt = _rb(jnp.dot(xs, wg[:, cols], preferred_element_type=f32))
        gt = _rb(gt * _rb(jax.nn.sigmoid(gt)))
        up = _rb(jnp.dot(xs, wu[:, cols], preferred_element_type=f32))
        acc = acc + jnp.dot((gt * up).astype(bf16), wd[cols, :], preferred_element_type=f32)
    yf = _rb(acc)
    for k, (idx, m) in enumerate(((i0, m0), (i1, m1))):
        row = pl.ds(idx, 1)
        n = get_row(xn, idx)
        upd = _rb(yf[k:k + 1, :] * _rb(jax.nn.sigmoid(m)))
        dl = _rb(n + upd) - n
        ob[row, :] = ob[row, :] + dl
    for i in range(NB - 2):
        for c in out_cps(i):
            c.start()
    mm2(NB - 2, h0)
    scan(bu1, h1)
    for c in out_cps(NB - 2):
        c.start()
    for q in range(2):
        mm2(NB - 1, h1, 4 * q, 4 * q + 4)
        last_cp(q).start()
    for i in range(NB - 1):
        for c in out_cps(i):
            c.wait()
    for q in range(2):
        last_cp(q).wait()


@jax.jit
def pallas_parallel_sum__ssm_conv_s5__moe_arch_mod__prompt_kernel(
    A_x, A_Lambda_re, A_Lambda_im, A_B_re, A_B_im, A_C_re, A_C_im, A_log_dt, A_Dskip,
    B_x, B_w_r, B_w_gate, B_w_up, B_w_down,
):
    hbm = pl.BlockSpec(memory_space=pl.ANY)
    vm = pl.BlockSpec(memory_space=pltpu.VMEM)
    row = lambda v: v.reshape(1, -1)
    out = pl.pallas_call(
        _kernel,
        out_shape=jax.ShapeDtypeStruct((L, D), f32),
        in_specs=[hbm, vm, vm, hbm, hbm, hbm, hbm, vm, vm, vm, hbm, hbm, hbm],
        out_specs=hbm,
        scratch_shapes=[
            pltpu.VMEM((L, D), bf16), pltpu.VMEM((G, NB * TP, 128), f32), pltpu.VMEM((T, D), bf16),
            pltpu.VMEM((T, D), bf16), pltpu.VMEM((L, D), f32),
            pltpu.VMEM((G, TP, 128), f32),
            pltpu.VMEM((2, P, D), bf16), pltpu.VMEM((2, D, P), bf16),
            pltpu.VMEM((D, F), bf16), pltpu.VMEM((D, F), bf16), pltpu.VMEM((F, D), bf16),
            pltpu.VMEM((2, T, P), f32), pltpu.VMEM((2, T, P), f32),
            pltpu.VMEM((2, T, P), bf16), pltpu.VMEM((2, T, P), bf16),
            pltpu.VMEM((L, 1), f32), pltpu.VMEM((12, 8, P), f32),
            pltpu.SemaphoreType.DMA((NB + 7,)), pltpu.SemaphoreType.DMA((NB + 1,)),
        ],
        compiler_params=pltpu.CompilerParams(vmem_limit_bytes=110 * 1024 * 1024),
    )(A_x.reshape(L, D), row(A_Lambda_re), row(A_Lambda_im), A_B_re, A_B_im, A_C_re, A_C_im,
      row(A_log_dt), row(A_Dskip), row(B_w_r), B_w_gate, B_w_up, B_w_down)
    return out.reshape(1, L, D)
```

```python
import jax
import jax.numpy as jnp
from jax import lax
import jax.experimental.pallas as pl
import jax.experimental.pallas.tpu as pltpu

L, D, P, F = 2048, 1024, 1024, 3584
T = 256
J = T // 8
NB = L // T
JP = J + 1
TP = 8 * JP
G = P // 128
FC = 512
NF = F // FC
f32, bf16 = jnp.float32, jnp.bfloat16
NT = (((1,), (1,)), ((), ()))


def _rb(v):
    return v.astype(bf16).astype(f32)


def _kernel(x_hbm, lre_ref, lim_ref, bre_hbm, bim_hbm, cre_hbm, cim_hbm, ldt_ref, dsk_ref,
            wr_ref, wg_hbm, wu_hbm, wd_hbm, o_hbm,
            xb, xn, xp0, xp1, ob, yb, bw, cw, wg, wu, wd, bu0, bu1, h0, h1, rr, st, sem, osem):
    def cp(src, dst, k):
        return pltpu.make_async_copy(src, dst, sem.at[k])

    x_cp = [cp(x_hbm.at[pl.ds(i * T, T)], xb.at[pl.ds(i * T, T)], i) for i in range(NB)]
    HP = P // 2
    b_cp = [cp(src.at[pl.ds(k * HP, HP)], bw.at[c, pl.ds(k * HP, HP)], NB + 7 + 2 * c + k)
            for c, src in enumerate((bre_hbm, bim_hbm)) for k in range(2)]
    c_cp = [cp(cre_hbm, cw.at[0], NB + 2), cp(cim_hbm, cw.at[1], NB + 3)]
    w_cp = [cp(wg_hbm, wg, NB + 4), cp(wu_hbm, wu, NB + 5), cp(wd_hbm, wd, NB + 6)]
    for c in x_cp[:1] + b_cp[:1]:
        c.start()

    lre = lre_ref[...].astype(f32)
    lim = lim_ref[...].astype(f32)
    dt = _rb(jnp.exp(ldt_ref[...].astype(f32)))
    ar, ai = dt * lre, dt * lim
    mag = jnp.exp(ar)
    lbr, lbi = mag * jnp.cos(ai), mag * jnp.sin(ai)
    den = lre * lre + lim * lim
    cfr = ((lbr - 1.0) * lre + lbi * lim) / den
    cfi = (lbi * lre - (lbr - 1.0) * lim) / den
    st[0] = jnp.broadcast_to(lbr, (8, P))
    st[1] = jnp.broadcast_to(lbi, (8, P))
    sub = lax.broadcasted_iota(jnp.int32, (8, P), 0)
    for k in range(3):
        n = float(J * (1 << k))
        m = jnp.exp(ar * n)
        keep = sub >= (1 << k)
        st[2 + 2 * k] = jnp.where(keep, jnp.broadcast_to(m * jnp.cos(ai * n), (8, P)), 0.0)
        st[3 + 2 * k] = jnp.where(keep, jnp.broadcast_to(m * jnp.sin(ai * n), (8, P)), 0.0)
    st[10] = jnp.broadcast_to(2.0 * cfr, (8, P))
    st[11] = jnp.broadcast_to(2.0 * cfi, (8, P))
    st[8] = jnp.zeros((8, P), f32)
    st[9] = jnp.zeros((8, P), f32)

    dsk = dsk_ref[...].astype(f32)
    dsk1 = dsk + 1.0
    wr = wr_ref[...].astype(f32)

    def lnorm(i, xp):
        for q in range(8):
            rows = pl.ds(i * T + q * J, J)
            x = xb[rows, :].astype(f32)
            mu = jnp.mean(x, axis=-1, keepdims=True)
            c = x - mu
            var = _rb(jnp.mean(c * c, axis=-1, keepdims=True))
            s = _rb(jnp.sqrt(_rb(var + 1e-5)))
            n = _rb(_rb(x - _rb(mu)) * (1.0 / s))
            base = x + n * dsk1
            for g in range(G):
                xn[g, pl.ds(i * TP + q * JP, J), :] = n[:, g * 128:(g + 1) * 128]
            ob[rows, :] = base
            rr[rows, :] = _rb(jnp.sum(n * wr, axis=-1, keepdims=True))
        for j in range(0, J, 2):
            for g in range(G):
                a = xn[g, pl.ds(i * TP + j, 8, stride=JP), :]
                b = xn[g, pl.ds(i * TP + j + 1, 8, stride=JP), :]
                xp[pl.ds(j * 8, 16), pl.ds(g * 128, 128)] = (
                    jnp.concatenate([a, b], axis=0).astype(bf16))

    def x_wait(i):
        rows = pl.ds(i * T, T)
        pltpu.make_async_copy(x_hbm.at[rows], xb.at[rows], sem.at[i]).wait()

    def mm1(xp, bu):
        xx = xp[...]
        bu[0] = lax.dot_general(xx, bw[0], NT, preferred_element_type=f32)
        bu[1] = lax.dot_general(xx, bw[1], NT, preferred_element_type=f32)

    def scan(bu, h):
        for g in range(G):
            ln_ = pl.ds(g * 128, 128)
            a_r, a_i = st[0, :, ln_], st[1, :, ln_]
            k_r, k_i = st[10, :, ln_], st[11, :, ln_]
            c_r, c_i = st[8, :, ln_], st[9, :, ln_]
            sr, si = c_r, c_i
            for j in range(J):
                rows = pl.ds(j * 8, 8)
                sr, si = (a_r * sr - a_i * si + bu[0, rows, ln_],
                          a_r * si + a_i * sr + bu[1, rows, ln_])
            for k in range(3):
                pr, pi = st[2 + 2 * k, :, ln_], st[3 + 2 * k, :, ln_]
                qr, qi = pltpu.roll(sr, 1 << k, 0), pltpu.roll(si, 1 << k, 0)
                sr, si = sr + (pr * qr - pi * qi), si + (pr * qi + pi * qr)
            er, ei = pltpu.roll(sr, 1, 0), pltpu.roll(si, 1, 0)
            first = lax.broadcasted_iota(jnp.int32, (8, 128), 0) == 0
            st[8, :, ln_] = jnp.where(first, er, 0.0)
            st[9, :, ln_] = jnp.where(first, ei, 0.0)
            sr, si = jnp.where(first, c_r, er), jnp.where(first, c_i, ei)
            for j in range(0, J, 2):
                o = []
                for jj in (j, j + 1):
                    rows = pl.ds(jj * 8, 8)
                    sr, si = (a_r * sr - a_i * si + bu[0, rows, ln_],
                              a_r * si + a_i * sr + bu[1, rows, ln_])
                    o.append((sr * k_r - si * k_i, (-sr) * k_i - si * k_r))
                rows = pl.ds(j * 8, 16)
                h[0, rows, ln_] = jnp.concatenate([o[0][0], o[1][0]], 0).astype(bf16)
                h[1, rows, ln_] = jnp.concatenate([o[0][1], o[1][1]], 0).astype(bf16)

    def mm2(i, h, g0=0, g1=G):
        wrows = pl.ds(g0 * 128, (g1 - g0) * 128)
        y = (lax.dot_general(h[0], cw[0, wrows, :], NT, preferred_element_type=f32)
             + lax.dot_general(h[1], cw[1, wrows, :], NT, preferred_element_type=f32))
        for j in range(J):
            for g in range(g0, g1):
                yb[g, pl.ds(j, 8, stride=JP), :] = (
                    y[j * 8:(j + 1) * 8, (g - g0) * 128:(g - g0 + 1) * 128])
        for q in range(8):
            rows = pl.ds(i * T + q * J, J)
            for g in range(g0, g1):
                cols = pl.ds(g * 128, 128)
                ob[rows, cols] = ob[rows, cols] + yb[g, pl.ds(q * JP, J), :]

    def last_cp(q):
        rows, cols = pl.ds((NB - 1) * T, T), pl.ds(q * 512, 512)
        return pltpu.make_async_copy(ob.at[rows, cols], o_hbm.at[rows, cols], osem.at[NB - 1 + q])

    def out_cps(i):
        rows = pl.ds(i * T, T)
        return [pltpu.make_async_copy(ob.at[rows], o_hbm.at[rows], osem.at[i])]

    def get_row(ref, idx):
        return jnp.concatenate([ref[g, pl.ds(idx + idx // J, 1), :] for g in range(G)], axis=1)

    x_wait(0)
    def mm1_part(c, k):
        w = pl.ds(k * HP, HP)
        bu0[c, :, w] = lax.dot_general(xp0[...], bw[c, w, :], NT, preferred_element_type=f32)

    b_cp[1].start()
    lnorm(0, xp0)
    b_cp[0].wait()
    b_cp[2].start()
    mm1_part(0, 0)
    b_cp[1].wait()
    b_cp[3].start()
    x_cp[1].start()
    mm1_part(0, 1)
    b_cp[2].wait()
    x_cp[2].start()
    mm1_part(1, 0)
    b_cp[3].wait()
    x_wait(1)
    for c in c_cp + x_cp[3:4]:
        c.start()
    lnorm(1, xp1)
    mm1_part(1, 1)
    x_wait(2)
    lnorm(2, xp0)
    mm1(xp1, bu1)
    scan(bu0, h0)
    for c in c_cp:
        c.wait()
    for c in x_cp[4:] + w_cp:
        c.start()

    def body(k, _):
        i = 2 * k
        x_wait(i + 3)
        lnorm(i + 3, xp1)
        mm2(i, h0)
        scan(bu1, h1)
        mm1(xp0, bu0)
        x_wait(i + 4)
        lnorm(i + 4, xp0)
        mm2(i + 1, h1)
        scan(bu0, h0)
        mm1(xp1, bu1)
        return 0
    for k in range(NB // 2 - 2):
        body(k, 0)
    x_wait(NB - 1)
    lnorm(NB - 1, xp1)
    mm2(NB - 4, h0)
    scan(bu1, h1)
    mm1(xp0, bu0)
    r = rr[...]
    ti = lax.broadcasted_iota(jnp.int32, (L, 1), 0)
    m0 = jnp.max(r, axis=0, keepdims=True)
    i0v = jnp.min(jnp.where(r == m0, ti, L), axis=0, keepdims=True)
    r2 = jnp.where(ti == i0v, -jnp.inf, r)
    m1 = jnp.max(r2, axis=0, keepdims=True)
    i1v = jnp.min(jnp.where((r2 == m1) & (ti != i0v), ti, L), axis=0, keepdims=True)
    i0 = jnp.clip(i0v[0, 0], 0, L - 1)
    i1 = jnp.clip(i1v[0, 0], 0, L - 1)

    for c in w_cp:
        c.wait()
    mm2(NB - 3, h1)
    scan(bu0, h0)
    mm1(xp1, bu1)
    s8 = lax.broadcasted_iota(jnp.int32, (16, D), 0)
    xs = jnp.where(s8 == 0, get_row(xn, i0), jnp.where(s8 == 1, get_row(xn, i1), 0.0)).astype(bf16)
    acc = jnp.zeros((16, D), f32)
    for c in range(NF):
        cols = pl.ds(c * FC, FC)
        gt = _rb(jnp.dot(xs, wg[:, cols], preferred_element_type=f32))
        gt = _rb(gt * _rb(jax.nn.sigmoid(gt)))
        up = _rb(jnp.dot(xs, wu[:, cols], preferred_element_type=f32))
        acc = acc + jnp.dot((gt * up).astype(bf16), wd[cols, :], preferred_element_type=f32)
    yf = _rb(acc)
    for k, (idx, m) in enumerate(((i0, m0), (i1, m1))):
        row = pl.ds(idx, 1)
        n = get_row(xn, idx)
        upd = _rb(yf[k:k + 1, :] * _rb(jax.nn.sigmoid(m)))
        dl = _rb(n + upd) - n
        ob[row, :] = ob[row, :] + dl
    for i in range(NB - 2):
        for c in out_cps(i):
            c.start()
    mm2(NB - 2, h0)
    scan(bu1, h1)
    for c in out_cps(NB - 2):
        c.start()
    for q in range(2):
        mm2(NB - 1, h1, 4 * q, 4 * q + 4)
        last_cp(q).start()
    for i in range(NB - 1):
        for c in out_cps(i):
            c.wait()
    for q in range(2):
        last_cp(q).wait()


@jax.jit
def pallas_parallel_sum__ssm_conv_s5__moe_arch_mod__prompt_kernel(
    A_x, A_Lambda_re, A_Lambda_im, A_B_re, A_B_im, A_C_re, A_C_im, A_log_dt, A_Dskip,
    B_x, B_w_r, B_w_gate, B_w_up, B_w_down,
):
    hbm = pl.BlockSpec(memory_space=pl.ANY)
    vm = pl.BlockSpec(memory_space=pltpu.VMEM)
    row = lambda v: v.reshape(1, -1)
    out = pl.pallas_call(
        _kernel,
        out_shape=jax.ShapeDtypeStruct((L, D), f32),
        in_specs=[hbm, vm, vm, hbm, hbm, hbm, hbm, vm, vm, vm, hbm, hbm, hbm],
        out_specs=hbm,
        scratch_shapes=[
            pltpu.VMEM((L, D), bf16), pltpu.VMEM((G, NB * TP, 128), f32), pltpu.VMEM((T, D), bf16),
            pltpu.VMEM((T, D), bf16), pltpu.VMEM((L, D), f32),
            pltpu.VMEM((G, TP, 128), f32),
            pltpu.VMEM((2, P, D), bf16), pltpu.VMEM((2, D, P), bf16),
            pltpu.VMEM((D, F), bf16), pltpu.VMEM((D, F), bf16), pltpu.VMEM((F, D), bf16),
            pltpu.VMEM((2, T, P), f32), pltpu.VMEM((2, T, P), f32),
            pltpu.VMEM((2, T, P), bf16), pltpu.VMEM((2, T, P), bf16),
            pltpu.VMEM((L, 1), f32), pltpu.VMEM((12, 8, P), f32),
            pltpu.SemaphoreType.DMA((NB + 11,)), pltpu.SemaphoreType.DMA((NB + 1,)),
        ],
        compiler_params=pltpu.CompilerParams(vmem_limit_bytes=110 * 1024 * 1024,
            flags={'XLA_TPU_EVENLY_DISTRIBUTE_CRITICAL_NODES': True}),
    )(A_x.reshape(L, D), row(A_Lambda_re), row(A_Lambda_im), A_B_re, A_B_im, A_C_re, A_C_im,
      row(A_log_dt), row(A_Dskip), row(B_w_r), B_w_gate, B_w_up, B_w_down)
    return out.reshape(1, L, D)
```

```python
import jax
import jax.numpy as jnp
from jax import lax
import jax.experimental.pallas as pl
import jax.experimental.pallas.tpu as pltpu

L, D, P, F = 2048, 1024, 1024, 3584
T = 256
J = T // 8
NB = L // T
JP = J + 1
TP = 8 * JP
G = P // 128
FC = 512
NF = F // FC
f32, bf16 = jnp.float32, jnp.bfloat16
NT = (((1,), (1,)), ((), ()))


def _rb(v):
    return v.astype(bf16).astype(f32)


def _kernel(x_hbm, lre_ref, lim_ref, bre_hbm, bim_hbm, cre_hbm, cim_hbm, ldt_ref, dsk_ref,
            wr_ref, wg_hbm, wu_hbm, wd_hbm, o_hbm,
            xb, xn, xp0, xp1, ob, yb, bw, cw, wg, wu, wd, bu0, bu1, h0, h1, rr, st, sem, osem):
    def cp(src, dst, k):
        return pltpu.make_async_copy(src, dst, sem.at[k])

    x_cp = [cp(x_hbm.at[pl.ds(i * T, T)], xb.at[pl.ds(i * T, T)], i) for i in range(NB)]
    HP = P // 2
    b_cp = [cp(src.at[pl.ds(k * HP, HP)], bw.at[c, pl.ds(k * HP, HP)], NB + 7 + 2 * c + k)
            for c, src in enumerate((bre_hbm, bim_hbm)) for k in range(2)]
    c_cp = [cp(cre_hbm, cw.at[0], NB + 2), cp(cim_hbm, cw.at[1], NB + 3)]
    w_cp = [cp(wg_hbm, wg, NB + 4), cp(wu_hbm, wu, NB + 5), cp(wd_hbm, wd, NB + 6)]
    for c in x_cp[:1] + b_cp[:1]:
        c.start()

    lre = lre_ref[...].astype(f32).reshape(1, -1)
    lim = lim_ref[...].astype(f32).reshape(1, -1)
    dt = _rb(jnp.exp(ldt_ref[...].astype(f32).reshape(1, -1)))
    ar, ai = dt * lre, dt * lim
    mag = jnp.exp(ar)
    lbr, lbi = mag * jnp.cos(ai), mag * jnp.sin(ai)
    den = lre * lre + lim * lim
    cfr = ((lbr - 1.0) * lre + lbi * lim) / den
    cfi = (lbi * lre - (lbr - 1.0) * lim) / den
    st[0] = jnp.broadcast_to(lbr, (8, P))
    st[1] = jnp.broadcast_to(lbi, (8, P))
    sub = lax.broadcasted_iota(jnp.int32, (8, P), 0)
    for k in range(3):
        n = float(J * (1 << k))
        m = jnp.exp(ar * n)
        keep = sub >= (1 << k)
        st[2 + 2 * k] = jnp.where(keep, jnp.broadcast_to(m * jnp.cos(ai * n), (8, P)), 0.0)
        st[3 + 2 * k] = jnp.where(keep, jnp.broadcast_to(m * jnp.sin(ai * n), (8, P)), 0.0)
    st[10] = jnp.broadcast_to(2.0 * cfr, (8, P))
    st[11] = jnp.broadcast_to(2.0 * cfi, (8, P))
    st[8] = jnp.zeros((8, P), f32)
    st[9] = jnp.zeros((8, P), f32)

    dsk = dsk_ref[...].astype(f32).reshape(1, -1)
    dsk1 = dsk + 1.0
    wr = wr_ref[...].astype(f32).reshape(1, -1)

    def lnorm(i, xp):
        for q in range(8):
            rows = pl.ds(i * T + q * J, J)
            x = xb[rows, :].astype(f32)
            mu = jnp.mean(x, axis=-1, keepdims=True)
            c = x - mu
            var = _rb(jnp.mean(c * c, axis=-1, keepdims=True))
            s = _rb(jnp.sqrt(_rb(var + 1e-5)))
            n = _rb(_rb(x - _rb(mu)) * (1.0 / s))
            base = x + n * dsk1
            for g in range(G):
                xn[g, pl.ds(i * TP + q * JP, J), :] = n[:, g * 128:(g + 1) * 128]
            ob[rows, :] = base
            rr[rows, :] = _rb(jnp.sum(n * wr, axis=-1, keepdims=True))
        for j in range(0, J, 2):
            for g in range(G):
                a = xn[g, pl.ds(i * TP + j, 8, stride=JP), :]
                b = xn[g, pl.ds(i * TP + j + 1, 8, stride=JP), :]
                xp[pl.ds(j * 8, 16), pl.ds(g * 128, 128)] = (
                    jnp.concatenate([a, b], axis=0).astype(bf16))

    def x_wait(i):
        rows = pl.ds(i * T, T)
        pltpu.make_async_copy(x_hbm.at[rows], xb.at[rows], sem.at[i]).wait()

    def mm1(xp, bu):
        xx = xp[...]
        bu[0] = lax.dot_general(xx, bw[0], NT, preferred_element_type=f32)
        bu[1] = lax.dot_general(xx, bw[1], NT, preferred_element_type=f32)

    def scan(bu, h):
        for g in range(G):
            ln_ = pl.ds(g * 128, 128)
            a_r, a_i = st[0, :, ln_], st[1, :, ln_]
            k_r, k_i = st[10, :, ln_], st[11, :, ln_]
            c_r, c_i = st[8, :, ln_], st[9, :, ln_]
            sr, si = c_r, c_i
            for j in range(J):
                rows = pl.ds(j * 8, 8)
                sr, si = (a_r * sr - a_i * si + bu[0, rows, ln_],
                          a_r * si + a_i * sr + bu[1, rows, ln_])
            for k in range(3):
                pr, pi = st[2 + 2 * k, :, ln_], st[3 + 2 * k, :, ln_]
                qr, qi = pltpu.roll(sr, 1 << k, 0), pltpu.roll(si, 1 << k, 0)
                sr, si = sr + (pr * qr - pi * qi), si + (pr * qi + pi * qr)
            er, ei = pltpu.roll(sr, 1, 0), pltpu.roll(si, 1, 0)
            first = lax.broadcasted_iota(jnp.int32, (8, 128), 0) == 0
            st[8, :, ln_] = jnp.where(first, er, 0.0)
            st[9, :, ln_] = jnp.where(first, ei, 0.0)
            sr, si = jnp.where(first, c_r, er), jnp.where(first, c_i, ei)
            for j in range(0, J, 2):
                o = []
                for jj in (j, j + 1):
                    rows = pl.ds(jj * 8, 8)
                    sr, si = (a_r * sr - a_i * si + bu[0, rows, ln_],
                              a_r * si + a_i * sr + bu[1, rows, ln_])
                    o.append((sr * k_r - si * k_i, (-sr) * k_i - si * k_r))
                rows = pl.ds(j * 8, 16)
                h[0, rows, ln_] = jnp.concatenate([o[0][0], o[1][0]], 0).astype(bf16)
                h[1, rows, ln_] = jnp.concatenate([o[0][1], o[1][1]], 0).astype(bf16)

    def mm2(i, h, g0=0, g1=G):
        wrows = pl.ds(g0 * 128, (g1 - g0) * 128)
        y = (lax.dot_general(h[0], cw[0, wrows, :], NT, preferred_element_type=f32)
             + lax.dot_general(h[1], cw[1, wrows, :], NT, preferred_element_type=f32))
        for j in range(J):
            for g in range(g0, g1):
                yb[g, pl.ds(j, 8, stride=JP), :] = (
                    y[j * 8:(j + 1) * 8, (g - g0) * 128:(g - g0 + 1) * 128])
        for q in range(8):
            rows = pl.ds(i * T + q * J, J)
            for g in range(g0, g1):
                cols = pl.ds(g * 128, 128)
                ob[rows, cols] = ob[rows, cols] + yb[g, pl.ds(q * JP, J), :]

    def last_cp(q):
        rows, cols = pl.ds((NB - 1) * T, T), pl.ds(q * 512, 512)
        return pltpu.make_async_copy(ob.at[rows, cols], o_hbm.at[rows, cols], osem.at[NB - 1 + q])

    def out_cps(i):
        rows = pl.ds(i * T, T)
        return [pltpu.make_async_copy(ob.at[rows], o_hbm.at[rows], osem.at[i])]

    def get_row(ref, idx):
        return jnp.concatenate([ref[g, pl.ds(idx + idx // J, 1), :] for g in range(G)], axis=1)

    x_wait(0)
    def mm1_part(c, k):
        w = pl.ds(k * HP, HP)
        bu0[c, :, w] = lax.dot_general(xp0[...], bw[c, w, :], NT, preferred_element_type=f32)

    b_cp[1].start()
    lnorm(0, xp0)
    b_cp[0].wait()
    b_cp[2].start()
    mm1_part(0, 0)
    b_cp[1].wait()
    b_cp[3].start()
    x_cp[1].start()
    mm1_part(0, 1)
    b_cp[2].wait()
    x_cp[2].start()
    mm1_part(1, 0)
    b_cp[3].wait()
    x_wait(1)
    for c in c_cp + x_cp[3:4]:
        c.start()
    lnorm(1, xp1)
    mm1_part(1, 1)
    x_wait(2)
    lnorm(2, xp0)
    mm1(xp1, bu1)
    scan(bu0, h0)
    for c in c_cp:
        c.wait()
    for c in x_cp[4:] + w_cp:
        c.start()

    def body(k, _):
        i = 2 * k
        x_wait(i + 3)
        lnorm(i + 3, xp1)
        mm2(i, h0)
        scan(bu1, h1)
        mm1(xp0, bu0)
        x_wait(i + 4)
        lnorm(i + 4, xp0)
        mm2(i + 1, h1)
        scan(bu0, h0)
        mm1(xp1, bu1)
        return 0
    for k in range(NB // 2 - 2):
        body(k, 0)
    x_wait(NB - 1)
    lnorm(NB - 1, xp1)
    mm2(NB - 4, h0)
    scan(bu1, h1)
    mm1(xp0, bu0)
    r = rr[...]
    ti = lax.broadcasted_iota(jnp.int32, (L, 1), 0)
    m0 = jnp.max(r, axis=0, keepdims=True)
    i0v = jnp.min(jnp.where(r == m0, ti, L), axis=0, keepdims=True)
    r2 = jnp.where(ti == i0v, -jnp.inf, r)
    m1 = jnp.max(r2, axis=0, keepdims=True)
    i1v = jnp.min(jnp.where((r2 == m1) & (ti != i0v), ti, L), axis=0, keepdims=True)
    i0 = jnp.clip(i0v[0, 0], 0, L - 1)
    i1 = jnp.clip(i1v[0, 0], 0, L - 1)

    for c in w_cp:
        c.wait()
    mm2(NB - 3, h1)
    scan(bu0, h0)
    mm1(xp1, bu1)
    s8 = lax.broadcasted_iota(jnp.int32, (16, D), 0)
    xs = jnp.where(s8 == 0, get_row(xn, i0), jnp.where(s8 == 1, get_row(xn, i1), 0.0)).astype(bf16)
    acc = jnp.zeros((16, D), f32)
    for c in range(NF):
        cols = pl.ds(c * FC, FC)
        gt = _rb(jnp.dot(xs, wg[:, cols], preferred_element_type=f32))
        gt = _rb(gt * _rb(jax.nn.sigmoid(gt)))
        up = _rb(jnp.dot(xs, wu[:, cols], preferred_element_type=f32))
        acc = acc + jnp.dot((gt * up).astype(bf16), wd[cols, :], preferred_element_type=f32)
    yf = _rb(acc)
    for k, (idx, m) in enumerate(((i0, m0), (i1, m1))):
        row = pl.ds(idx, 1)
        n = get_row(xn, idx)
        upd = _rb(yf[k:k + 1, :] * _rb(jax.nn.sigmoid(m)))
        dl = _rb(n + upd) - n
        ob[row, :] = ob[row, :] + dl
    for i in range(NB - 2):
        for c in out_cps(i):
            c.start()
    mm2(NB - 2, h0)
    scan(bu1, h1)
    for c in out_cps(NB - 2):
        c.start()
    for q in range(2):
        mm2(NB - 1, h1, 4 * q, 4 * q + 4)
        last_cp(q).start()
    for i in range(NB - 1):
        for c in out_cps(i):
            c.wait()
    for q in range(2):
        last_cp(q).wait()


@jax.jit
def pallas_parallel_sum__ssm_conv_s5__moe_arch_mod__prompt_kernel(
    A_x, A_Lambda_re, A_Lambda_im, A_B_re, A_B_im, A_C_re, A_C_im, A_log_dt, A_Dskip,
    B_x, B_w_r, B_w_gate, B_w_up, B_w_down,
):
    hbm = pl.BlockSpec(memory_space=pl.ANY)
    vm = pl.BlockSpec(memory_space=pltpu.VMEM)
    row = lambda v: v
    out = pl.pallas_call(
        _kernel,
        out_shape=jax.ShapeDtypeStruct((L, D), f32),
        in_specs=[hbm, vm, vm, hbm, hbm, hbm, hbm, vm, vm, vm, hbm, hbm, hbm],
        out_specs=hbm,
        scratch_shapes=[
            pltpu.VMEM((L, D), bf16), pltpu.VMEM((G, NB * TP, 128), f32), pltpu.VMEM((T, D), bf16),
            pltpu.VMEM((T, D), bf16), pltpu.VMEM((L, D), f32),
            pltpu.VMEM((G, TP, 128), f32),
            pltpu.VMEM((2, P, D), bf16), pltpu.VMEM((2, D, P), bf16),
            pltpu.VMEM((D, F), bf16), pltpu.VMEM((D, F), bf16), pltpu.VMEM((F, D), bf16),
            pltpu.VMEM((2, T, P), f32), pltpu.VMEM((2, T, P), f32),
            pltpu.VMEM((2, T, P), bf16), pltpu.VMEM((2, T, P), bf16),
            pltpu.VMEM((L, 1), f32), pltpu.VMEM((12, 8, P), f32),
            pltpu.SemaphoreType.DMA((NB + 11,)), pltpu.SemaphoreType.DMA((NB + 1,)),
        ],
        compiler_params=pltpu.CompilerParams(vmem_limit_bytes=110 * 1024 * 1024,
            flags={'XLA_TPU_EVENLY_DISTRIBUTE_CRITICAL_NODES': True}),
    )(A_x.reshape(L, D), row(A_Lambda_re), row(A_Lambda_im), A_B_re, A_B_im, A_C_re, A_C_im,
      row(A_log_dt), row(A_Dskip), row(B_w_r), B_w_gate, B_w_up, B_w_down)
    return out.reshape(1, L, D)
```

```python
import jax
import jax.numpy as jnp
from jax import lax
import jax.experimental.pallas as pl
import jax.experimental.pallas.tpu as pltpu

L, D, P, F = 2048, 1024, 1024, 3584
T = 256
J = T // 8
NB = L // T
JP = J + 1
TP = 8 * JP
G = P // 128
FC = 896
NF = F // FC
f32, bf16 = jnp.float32, jnp.bfloat16
NT = (((1,), (1,)), ((), ()))


def _rb(v):
    return v.astype(bf16).astype(f32)


def _kernel(x_hbm, lre_ref, lim_ref, bre_hbm, bim_hbm, cre_hbm, cim_hbm, ldt_ref, dsk_ref,
            wr_ref, wg_hbm, wu_hbm, wd_hbm, o_hbm,
            xb, xn, xp0, xp1, ob, yb, bw, cw, wg, wu, wd, bu0, bu1, h0, h1, rr, st, sem, osem):
    def cp(src, dst, k):
        return pltpu.make_async_copy(src, dst, sem.at[k])

    x_cp = [cp(x_hbm.at[pl.ds(i * T, T)], xb.at[pl.ds(i * T, T)], i) for i in range(NB)]
    HP = P // 2
    b_cp = [cp(src.at[pl.ds(k * HP, HP)], bw.at[c, pl.ds(k * HP, HP)], NB + 7 + 2 * c + k)
            for c, src in enumerate((bre_hbm, bim_hbm)) for k in range(2)]
    c_cp = [cp(cre_hbm, cw.at[0], NB + 2), cp(cim_hbm, cw.at[1], NB + 3)]
    w_cp = [cp(wg_hbm, wg, NB + 4), cp(wu_hbm, wu, NB + 5), cp(wd_hbm, wd, NB + 6)]
    for c in x_cp[:1] + b_cp[:1]:
        c.start()

    lre = lre_ref[...].astype(f32).reshape(1, -1)
    lim = lim_ref[...].astype(f32).reshape(1, -1)
    dt = _rb(jnp.exp(ldt_ref[...].astype(f32).reshape(1, -1)))
    ar, ai = dt * lre, dt * lim
    mag = jnp.exp(ar)
    lbr, lbi = mag * jnp.cos(ai), mag * jnp.sin(ai)
    den = lre * lre + lim * lim
    cfr = ((lbr - 1.0) * lre + lbi * lim) / den
    cfi = (lbi * lre - (lbr - 1.0) * lim) / den
    st[0] = jnp.broadcast_to(lbr, (8, P))
    st[1] = jnp.broadcast_to(lbi, (8, P))
    sub = lax.broadcasted_iota(jnp.int32, (8, P), 0)
    for k in range(3):
        n = float(J * (1 << k))
        m = jnp.exp(ar * n)
        keep = sub >= (1 << k)
        st[2 + 2 * k] = jnp.where(keep, jnp.broadcast_to(m * jnp.cos(ai * n), (8, P)), 0.0)
        st[3 + 2 * k] = jnp.where(keep, jnp.broadcast_to(m * jnp.sin(ai * n), (8, P)), 0.0)
    st[10] = jnp.broadcast_to(2.0 * cfr, (8, P))
    st[11] = jnp.broadcast_to(2.0 * cfi, (8, P))
    st[8] = jnp.zeros((8, P), f32)
    st[9] = jnp.zeros((8, P), f32)

    dsk = dsk_ref[...].astype(f32).reshape(1, -1)
    dsk1 = dsk + 1.0
    rr[...] = jnp.full((J, 128), -jnp.inf, f32)
    wr = wr_ref[...].astype(f32).reshape(1, -1)

    def lnorm(i, xp):
        for q in range(8):
            rows = pl.ds(i * T + q * J, J)
            x = xb[rows, :].astype(f32)
            mu = jnp.mean(x, axis=-1, keepdims=True)
            c = x - mu
            var = _rb(jnp.mean(c * c, axis=-1, keepdims=True))
            s = _rb(jnp.sqrt(_rb(var + 1e-5)))
            n = _rb(_rb(x - _rb(mu)) * (1.0 / s))
            base = x + n * dsk1
            for g in range(G):
                xn[g, pl.ds(i * TP + q * JP, J), :] = n[:, g * 128:(g + 1) * 128]
            ob[rows, :] = base
            lane = lax.broadcasted_iota(jnp.int32, (J, 128), 1)
            rr[...] = jnp.where(lane == 8 * i + q, _rb(jnp.sum(n * wr, axis=-1, keepdims=True)), rr[...])
        for j in range(0, J, 2):
            for g in range(G):
                a = xn[g, pl.ds(i * TP + j, 8, stride=JP), :]
                b = xn[g, pl.ds(i * TP + j + 1, 8, stride=JP), :]
                xp[pl.ds(j * 8, 16), pl.ds(g * 128, 128)] = (
                    jnp.concatenate([a, b], axis=0).astype(bf16))

    def x_wait(i):
        rows = pl.ds(i * T, T)
        pltpu.make_async_copy(x_hbm.at[rows], xb.at[rows], sem.at[i]).wait()

    def mm1(xp, bu):
        xx = xp[...]
        bu[0] = lax.dot_general(xx, bw[0], NT, preferred_element_type=f32)
        bu[1] = lax.dot_general(xx, bw[1], NT, preferred_element_type=f32)

    def scan(bu, h):
        for g in range(G):
            ln_ = pl.ds(g * 128, 128)
            a_r, a_i = st[0, :, ln_], st[1, :, ln_]
            k_r, k_i = st[10, :, ln_], st[11, :, ln_]
            c_r, c_i = st[8, :, ln_], st[9, :, ln_]
            sr, si = c_r, c_i
            for j in range(J):
                rows = pl.ds(j * 8, 8)
                sr, si = (a_r * sr - a_i * si + bu[0, rows, ln_],
                          a_r * si + a_i * sr + bu[1, rows, ln_])
            for k in range(3):
                pr, pi = st[2 + 2 * k, :, ln_], st[3 + 2 * k, :, ln_]
                qr, qi = pltpu.roll(sr, 1 << k, 0), pltpu.roll(si, 1 << k, 0)
                sr, si = sr + (pr * qr - pi * qi), si + (pr * qi + pi * qr)
            er, ei = pltpu.roll(sr, 1, 0), pltpu.roll(si, 1, 0)
            first = lax.broadcasted_iota(jnp.int32, (8, 128), 0) == 0
            st[8, :, ln_] = jnp.where(first, er, 0.0)
            st[9, :, ln_] = jnp.where(first, ei, 0.0)
            sr, si = jnp.where(first, c_r, er), jnp.where(first, c_i, ei)
            for j in range(0, J, 2):
                o = []
                for jj in (j, j + 1):
                    rows = pl.ds(jj * 8, 8)
                    sr, si = (a_r * sr - a_i * si + bu[0, rows, ln_],
                              a_r * si + a_i * sr + bu[1, rows, ln_])
                    o.append((sr * k_r - si * k_i, (-sr) * k_i - si * k_r))
                rows = pl.ds(j * 8, 16)
                h[0, rows, ln_] = jnp.concatenate([o[0][0], o[1][0]], 0).astype(bf16)
                h[1, rows, ln_] = jnp.concatenate([o[0][1], o[1][1]], 0).astype(bf16)

    def mm2(i, h, g0=0, g1=G):
        wrows = pl.ds(g0 * 128, (g1 - g0) * 128)
        y = (lax.dot_general(h[0], cw[0, wrows, :], NT, preferred_element_type=f32)
             + lax.dot_general(h[1], cw[1, wrows, :], NT, preferred_element_type=f32))
        for j in range(J):
            for g in range(g0, g1):
                yb[g, pl.ds(j, 8, stride=JP), :] = (
                    y[j * 8:(j + 1) * 8, (g - g0) * 128:(g - g0 + 1) * 128])
        for q in range(8):
            rows = pl.ds(i * T + q * J, J)
            for g in range(g0, g1):
                cols = pl.ds(g * 128, 128)
                ob[rows, cols] = ob[rows, cols] + yb[g, pl.ds(q * JP, J), :]

    def last_cp(q):
        rows, cols = pl.ds((NB - 1) * T, T), pl.ds(q * 512, 512)
        return pltpu.make_async_copy(ob.at[rows, cols], o_hbm.at[rows, cols], osem.at[NB - 1 + q])

    def out_cps(i):
        rows = pl.ds(i * T, T)
        return [pltpu.make_async_copy(ob.at[rows], o_hbm.at[rows], osem.at[i])]

    def get_row(ref, idx):
        return jnp.concatenate([ref[g, pl.ds(idx + idx // J, 1), :] for g in range(G)], axis=1)

    x_wait(0)
    def mm1_part(c, k):
        w = pl.ds(k * HP, HP)
        bu0[c, :, w] = lax.dot_general(xp0[...], bw[c, w, :], NT, preferred_element_type=f32)

    b_cp[1].start()
    lnorm(0, xp0)
    b_cp[0].wait()
    b_cp[2].start()
    mm1_part(0, 0)
    b_cp[1].wait()
    b_cp[3].start()
    x_cp[1].start()
    mm1_part(0, 1)
    b_cp[2].wait()
    x_cp[2].start()
    mm1_part(1, 0)
    b_cp[3].wait()
    x_wait(1)
    for c in c_cp + x_cp[3:4]:
        c.start()
    lnorm(1, xp1)
    mm1_part(1, 1)
    x_wait(2)
    lnorm(2, xp0)
    mm1(xp1, bu1)
    scan(bu0, h0)
    for c in c_cp:
        c.wait()
    for c in x_cp[4:] + w_cp:
        c.start()

    def body(k, _):
        i = 2 * k
        x_wait(i + 3)
        lnorm(i + 3, xp1)
        mm2(i, h0)
        scan(bu1, h1)
        mm1(xp0, bu0)
        x_wait(i + 4)
        lnorm(i + 4, xp0)
        mm2(i + 1, h1)
        scan(bu0, h0)
        mm1(xp1, bu1)
        return 0
    for k in range(NB // 2 - 2):
        body(k, 0)
    x_wait(NB - 1)
    lnorm(NB - 1, xp1)
    mm2(NB - 4, h0)
    scan(bu1, h1)
    mm1(xp0, bu0)
    for c in w_cp:
        c.wait()
    r = rr[...]
    lane = lax.broadcasted_iota(jnp.int32, (J, 128), 1)
    ti = jnp.where(lane < L // J, lane * J + lax.broadcasted_iota(jnp.int32, (J, 128), 0), L)

    def red(op, v):
        return op(op(v, axis=0, keepdims=True), axis=1, keepdims=True)

    m0 = red(jnp.max, r)
    i0v = red(jnp.min, jnp.where(r == m0, ti, L))
    r2 = jnp.where(ti == i0v, -jnp.inf, r)
    m1 = red(jnp.max, r2)
    i1v = red(jnp.min, jnp.where((r2 == m1) & (ti != i0v), ti, L))
    i0 = jnp.clip(i0v[0, 0], 0, L - 1)
    i1 = jnp.clip(i1v[0, 0], 0, L - 1)

    mm2(NB - 3, h1)
    scan(bu0, h0)
    mm1(xp1, bu1)
    s8 = lax.broadcasted_iota(jnp.int32, (16, D), 0)
    xs = jnp.where(s8 == 0, get_row(xn, i0), jnp.where(s8 == 1, get_row(xn, i1), 0.0)).astype(bf16)
    acc = jnp.zeros((16, D), f32)
    for c in range(NF):
        cols = pl.ds(c * FC, FC)
        gt = _rb(jnp.dot(xs, wg[:, cols], preferred_element_type=f32))
        gt = _rb(gt * _rb(jax.nn.sigmoid(gt)))
        up = _rb(jnp.dot(xs, wu[:, cols], preferred_element_type=f32))
        acc = acc + jnp.dot((gt * up).astype(bf16), wd[cols, :], preferred_element_type=f32)
    yf = _rb(acc)
    for k, (idx, m) in enumerate(((i0, m0), (i1, m1))):
        row = pl.ds(idx, 1)
        n = get_row(xn, idx)
        upd = _rb(yf[k:k + 1, :] * _rb(jax.nn.sigmoid(m)))
        dl = _rb(n + upd) - n
        ob[row, :] = ob[row, :] + dl
    for i in range(NB - 2):
        for c in out_cps(i):
            c.start()
    mm2(NB - 2, h0)
    scan(bu1, h1)
    for c in out_cps(NB - 2):
        c.start()
    for q in range(2):
        mm2(NB - 1, h1, 4 * q, 4 * q + 4)
        last_cp(q).start()
    for i in range(NB - 1):
        for c in out_cps(i):
            c.wait()
    for q in range(2):
        last_cp(q).wait()


@jax.jit
def pallas_parallel_sum__ssm_conv_s5__moe_arch_mod__prompt_kernel(
    A_x, A_Lambda_re, A_Lambda_im, A_B_re, A_B_im, A_C_re, A_C_im, A_log_dt, A_Dskip,
    B_x, B_w_r, B_w_gate, B_w_up, B_w_down,
):
    hbm = pl.BlockSpec(memory_space=pl.ANY)
    vm = pl.BlockSpec(memory_space=pltpu.VMEM)
    row = lambda v: v
    out = pl.pallas_call(
        _kernel,
        out_shape=jax.ShapeDtypeStruct((L, D), f32),
        in_specs=[hbm, vm, vm, hbm, hbm, hbm, hbm, vm, vm, vm, hbm, hbm, hbm],
        out_specs=hbm,
        scratch_shapes=[
            pltpu.VMEM((L, D), bf16), pltpu.VMEM((G, NB * TP, 128), f32), pltpu.VMEM((T, D), bf16),
            pltpu.VMEM((T, D), bf16), pltpu.VMEM((L, D), f32),
            pltpu.VMEM((G, TP, 128), f32),
            pltpu.VMEM((2, P, D), bf16), pltpu.VMEM((2, D, P), bf16),
            pltpu.VMEM((D, F), bf16), pltpu.VMEM((D, F), bf16), pltpu.VMEM((F, D), bf16),
            pltpu.VMEM((2, T, P), f32), pltpu.VMEM((2, T, P), f32),
            pltpu.VMEM((2, T, P), bf16), pltpu.VMEM((2, T, P), bf16),
            pltpu.VMEM((J, 128), f32), pltpu.VMEM((12, 8, P), f32),
            pltpu.SemaphoreType.DMA((NB + 11,)), pltpu.SemaphoreType.DMA((NB + 1,)),
        ],
        compiler_params=pltpu.CompilerParams(vmem_limit_bytes=110 * 1024 * 1024,
            flags={'XLA_TPU_EVENLY_DISTRIBUTE_CRITICAL_NODES': True}),
    )(A_x.reshape(L, D), row(A_Lambda_re), row(A_Lambda_im), A_B_re, A_B_im, A_C_re, A_C_im,
      row(A_log_dt), row(A_Dskip), row(B_w_r), B_w_gate, B_w_up, B_w_down)
    return out.reshape(1, L, D)
```

```python
import jax
import jax.numpy as jnp
from jax import lax
import jax.experimental.pallas as pl
import jax.experimental.pallas.tpu as pltpu

L, D, P, F = 2048, 1024, 1024, 3584
T = 256
J = T // 8
NB = L // T
JP = J + 1
TP = 8 * JP
G = P // 128
NC = 4
PC = P // NC
FC = 896
NF = F // FC
f32, bf16 = jnp.float32, jnp.bfloat16
NT = (((1,), (1,)), ((), ()))


def _rb(v):
    return v.astype(bf16).astype(f32)


def _lhs7(a11, a12, a21, a22):
    return (a11 + a22, a21 + a22, a11, a22, a11 + a12, a21 - a11, a12 - a22)


def _rhs7(b11, b12, b21, b22):
    return (b11 + b22, b11, b12 - b22, b21 - b11, b22, b11 + b12, b21 + b22)


def _out4(m):
    return (m[0] + m[3] - m[4] + m[6], m[2] + m[4], m[1] + m[3], m[0] - m[1] + m[2] + m[5])


def _kernel(x_hbm, lre_ref, lim_ref, bre_hbm, bim_hbm, cre_hbm, cim_hbm, ldt_ref, dsk_ref,
            wr_ref, wg_hbm, wu_hbm, wd_hbm, o_hbm,
            xb, xn, ob, yb, bw, cw, bq, cq, wg, wu, wd, rr, st, sem, osem, *rings):
    xq, bu, hq = rings[:4], rings[4:7], rings[7:]

    def cp(src, dst, k):
        return pltpu.make_async_copy(src, dst, sem.at[k])

    x_cp = [cp(x_hbm.at[pl.ds(i * T, T)], xb.at[pl.ds(i * T, T)], i) for i in range(NB)]
    b_cp = [[cp(src.at[pl.ds(k * PC, PC)], bw.at[c, pl.ds(k * PC, PC)], NB + 5 + 2 * k + c)
             for c, src in enumerate((bre_hbm, bim_hbm))] for k in range(NC)]
    c_cp = [cp(cre_hbm, cw.at[0], NB), cp(cim_hbm, cw.at[1], NB + 1)]
    w_cp = [cp(wg_hbm, wg, NB + 2), cp(wu_hbm, wu, NB + 3), cp(wd_hbm, wd, NB + 4)]

    def start(cs):
        for c in cs:
            c.start()

    def wait(cs):
        for c in cs:
            c.wait()

    start(x_cp[:1] + b_cp[0] + x_cp[1:2])

    lre = lre_ref[...].astype(f32).reshape(1, -1)
    lim = lim_ref[...].astype(f32).reshape(1, -1)
    dt = _rb(jnp.exp(ldt_ref[...].astype(f32).reshape(1, -1)))
    ar, ai = dt * lre, dt * lim
    mag = jnp.exp(ar)
    lbr, lbi = mag * jnp.cos(ai), mag * jnp.sin(ai)
    den = lre * lre + lim * lim
    cfr = ((lbr - 1.0) * lre + lbi * lim) / den
    cfi = (lbi * lre - (lbr - 1.0) * lim) / den
    st[0] = jnp.broadcast_to(lbr, (8, P))
    st[1] = jnp.broadcast_to(lbi, (8, P))
    sub = lax.broadcasted_iota(jnp.int32, (8, P), 0)
    for k in range(3):
        n = float(J * (1 << k))
        m = jnp.exp(ar * n)
        keep = sub >= (1 << k)
        st[2 + 2 * k] = jnp.where(keep, jnp.broadcast_to(m * jnp.cos(ai * n), (8, P)), 0.0)
        st[3 + 2 * k] = jnp.where(keep, jnp.broadcast_to(m * jnp.sin(ai * n), (8, P)), 0.0)
    st[8] = jnp.zeros((8, P), f32)
    st[9] = jnp.zeros((8, P), f32)

    dsk = dsk_ref[...].astype(f32).reshape(1, -1)
    dsk1 = dsk + 1.0
    rr[...] = jnp.full((J, 128), -jnp.inf, f32)
    wr = wr_ref[...].astype(f32).reshape(1, -1)

    def lnorm(i):
        for q in range(8):
            rows = pl.ds(i * T + q * J, J)
            x = xb[rows, :].astype(f32)
            mu = jnp.mean(x, axis=-1, keepdims=True)
            c = x - mu
            var = _rb(jnp.mean(c * c, axis=-1, keepdims=True))
            s = _rb(jnp.sqrt(_rb(var + 1e-5)))
            n = _rb(_rb(x - _rb(mu)) * (1.0 / s))
            base = x + n * dsk1
            for g in range(G):
                xn[g, pl.ds(i * TP + q * JP, J), :] = n[:, g * 128:(g + 1) * 128]
            ob[rows, :] = base
            lane = lax.broadcasted_iota(jnp.int32, (J, 128), 1)
            rr[...] = jnp.where(lane == 8 * i + q, _rb(jnp.sum(n * wr, axis=-1, keepdims=True)), rr[...])
        for j in range(0, J, 4):
            for g in range(G // 2):
                def ld(jj, gg):
                    return jnp.concatenate(
                        [xn[gg, pl.ds(i * TP + jj + e, 8, stride=JP), :] for e in (0, 2)], axis=0)
                ops = _lhs7(ld(j, g), ld(j, g + G // 2), ld(j + 1, g), ld(j + 1, g + G // 2))
                for m, v in enumerate(ops):
                    xq[i % 4][m, pl.ds(j * 4, 16), pl.ds(g * 128, 128)] = v.astype(bf16)

    def b_prep(k):
        for r0 in range(k * PC, (k + 1) * PC, 64):
            rows = pl.ds(r0, 64)
            lo, hi = pl.ds(0, D // 2), pl.ds(D // 2, D // 2)
            ops = _rhs7(bw[0, rows, lo].astype(f32), bw[1, rows, lo].astype(f32),
                        bw[0, rows, hi].astype(f32), bw[1, rows, hi].astype(f32))
            for m, v in enumerate(ops):
                bq[m, rows, :] = v.astype(bf16)

    def c_prep():
        kr, ki = 2.0 * cfr, 2.0 * cfi
        for r0 in range(0, D // 2, 16):
            w = []
            for rows in (pl.ds(r0, 16), pl.ds(D // 2 + r0, 16)):
                cr, ci = cw[0, rows, :].astype(f32), cw[1, rows, :].astype(f32)
                w.append((cr * kr - ci * ki, -(cr * ki) - ci * kr))
            for m, v in enumerate(_rhs7(w[0][0], w[1][0], w[0][1], w[1][1])):
                cq[m, pl.ds(r0, 16), :] = v.astype(bf16)

    def mm1(i, k0=0, k1=NC):
        w = pl.ds(k0 * PC, (k1 - k0) * PC)
        c = _out4([lax.dot_general(xq[i % 4][m], bq[m, w, :], NT, preferred_element_type=f32)
                   for m in range(7)])
        for par in range(2):
            for ri in range(2):
                bu[i % 3][ri, par, :, w] = c[2 * par + ri]

    def scan(i, k0=0, k1=NC):
        b, h = bu[i % 3], hq[i % 3]
        for g in range(k0 * PC // 128, k1 * PC // 128):
            ln_ = pl.ds(g * 128, 128)
            a_r, a_i = st[0, :, ln_], st[1, :, ln_]
            c_r, c_i = st[8, :, ln_], st[9, :, ln_]

            def adv(j, sr, si):
                rows = pl.ds((j // 2) * 8, 8)
                return (a_r * sr - a_i * si + b[0, j % 2, rows, ln_],
                        a_r * si + a_i * sr + b[1, j % 2, rows, ln_])

            sr, si = c_r, c_i
            for j in range(J):
                sr, si = adv(j, sr, si)
            for k in range(3):
                pr, pi = st[2 + 2 * k, :, ln_], st[3 + 2 * k, :, ln_]
                qr, qi = pltpu.roll(sr, 1 << k, 0), pltpu.roll(si, 1 << k, 0)
                sr, si = sr + (pr * qr - pi * qi), si + (pr * qi + pi * qr)
            er, ei = pltpu.roll(sr, 1, 0), pltpu.roll(si, 1, 0)
            first = lax.broadcasted_iota(jnp.int32, (8, 128), 0) == 0
            st[8, :, ln_] = jnp.where(first, er, 0.0)
            st[9, :, ln_] = jnp.where(first, ei, 0.0)
            sr, si = jnp.where(first, c_r, er), jnp.where(first, c_i, ei)
            for j in range(0, J, 4):
                o = []
                for jj in range(j, j + 4):
                    sr, si = adv(jj, sr, si)
                    o.append((sr, si))
                lo, hi = _lhs7(*o[0], *o[1]), _lhs7(*o[2], *o[3])
                for m in range(7):
                    h[m, pl.ds(j * 4, 16), ln_] = jnp.concatenate([lo[m], hi[m]], 0).astype(bf16)

    def mm2(i, g0=0, g1=G // 2):
        wrows = pl.ds(g0 * 128, (g1 - g0) * 128)
        c = _out4([lax.dot_general(hq[i % 3][m], cq[m, wrows, :], NT, preferred_element_type=f32)
                   for m in range(7)])
        for j in range(J):
            for half in range(2):
                for g in range(g0, g1):
                    yb[g + half * (G // 2), pl.ds(j, 8, stride=JP), :] = c[2 * (j % 2) + half][
                        (j // 2) * 8:(j // 2 + 1) * 8, (g - g0) * 128:(g - g0 + 1) * 128]
        for q in range(8):
            rows = pl.ds(i * T + q * J, J)
            for half in range(2):
                for g in range(g0 + half * (G // 2), g1 + half * (G // 2)):
                    cols = pl.ds(g * 128, 128)
                    ob[rows, cols] = ob[rows, cols] + yb[g, pl.ds(q * JP, J), :]

    def out_cp(i):
        rows = pl.ds(i * T, T)
        return pltpu.make_async_copy(ob.at[rows], o_hbm.at[rows], osem.at[i])

    def last_cp(q):
        rows = pl.ds((NB - 1) * T, T)
        return [pltpu.make_async_copy(ob.at[rows, cols], o_hbm.at[rows, cols], osem.at[NB - 1 + 2 * q + e])
                for e, cols in enumerate((pl.ds(q * 256, 256), pl.ds(D // 2 + q * 256, 256)))]

    def get_row(ref, idx):
        return jnp.concatenate([ref[g, pl.ds(idx + idx // J, 1), :] for g in range(G)], axis=1)

    wait(x_cp[:1])
    start(b_cp[1])
    lnorm(0)
    for k in range(NC):
        wait(b_cp[k] + (x_cp[1:2] if k == 0 else x_cp[k:k + 1] if k >= 2 else []))
        start((x_cp[2:3] + b_cp[2], x_cp[3:4] + b_cp[3], c_cp, x_cp[4:])[k])
        b_prep(k)
        mm1(0, k, k + 1)
        if k != 1:
            lnorm(max(k, 1))
        mm1(1, k, k + 1)
        if k > 0:
            scan(0, k - 1, k)
            scan(1, k - 1, k)
    wait(c_cp)
    start(w_cp)
    mm1(2)
    scan(0, NC - 1, NC)
    scan(1, NC - 1, NC)
    c_prep()
    for i in range(NB - 4):
        wait(x_cp[i + 4:i + 5])
        lnorm(i + 4)
        mm2(i)
        scan(i + 2)
        mm1(i + 3)
    wait(w_cp[:2])
    r = rr[...]
    lane = lax.broadcasted_iota(jnp.int32, (J, 128), 1)
    ti = jnp.where(lane < L // J, lane * J + lax.broadcasted_iota(jnp.int32, (J, 128), 0), L)

    def red(op, v):
        return op(op(v, axis=0, keepdims=True), axis=1, keepdims=True)

    m0 = red(jnp.max, r)
    i0v = red(jnp.min, jnp.where(r == m0, ti, L))
    r2 = jnp.where(ti == i0v, -jnp.inf, r)
    m1 = red(jnp.max, r2)
    i1v = red(jnp.min, jnp.where((r2 == m1) & (ti != i0v), ti, L))
    i0 = jnp.clip(i0v[0, 0], 0, L - 1)
    i1 = jnp.clip(i1v[0, 0], 0, L - 1)

    s8 = lax.broadcasted_iota(jnp.int32, (16, D), 0)
    xs = jnp.where(s8 == 0, get_row(xn, i0), jnp.where(s8 == 1, get_row(xn, i1), 0.0)).astype(bf16)
    mm2(NB - 4)
    scan(NB - 2)
    mm1(NB - 1)
    wait(w_cp[2:])
    mm2(NB - 3)
    scan(NB - 1)
    acc = jnp.zeros((16, D), f32)
    for c in range(NF):
        cols = pl.ds(c * FC, FC)
        gt = _rb(jnp.dot(xs, wg[:, cols], preferred_element_type=f32))
        gt = _rb(gt * _rb(jax.nn.sigmoid(gt)))
        up = _rb(jnp.dot(xs, wu[:, cols], preferred_element_type=f32))
        acc = acc + jnp.dot((gt * up).astype(bf16), wd[cols, :], preferred_element_type=f32)
    yf = _rb(acc)
    for k, (idx, m) in enumerate(((i0, m0), (i1, m1))):
        row = pl.ds(idx, 1)
        n = get_row(xn, idx)
        upd = _rb(yf[k:k + 1, :] * _rb(jax.nn.sigmoid(m)))
        dl = _rb(n + upd) - n
        ob[row, :] = ob[row, :] + dl
    start([out_cp(i) for i in range(NB - 2)])
    mm2(NB - 2)
    out_cp(0).wait()
    out_cp(NB - 2).start()
    for q in range(2):
        mm2(NB - 1, 2 * q, 2 * q + 2)
        start(last_cp(q))
    wait([out_cp(i) for i in range(1, NB - 1)] + last_cp(0) + last_cp(1))


@jax.jit
def pallas_parallel_sum__ssm_conv_s5__moe_arch_mod__prompt_kernel(
    A_x, A_Lambda_re, A_Lambda_im, A_B_re, A_B_im, A_C_re, A_C_im, A_log_dt, A_Dskip,
    B_x, B_w_r, B_w_gate, B_w_up, B_w_down,
):
    hbm = pl.BlockSpec(memory_space=pl.ANY)
    vm = pl.BlockSpec(memory_space=pltpu.VMEM)
    row = lambda v: v
    out = pl.pallas_call(
        _kernel,
        out_shape=jax.ShapeDtypeStruct((L, D), f32),
        in_specs=[hbm, vm, vm, hbm, hbm, hbm, hbm, vm, vm, vm, hbm, hbm, hbm],
        out_specs=hbm,
        scratch_shapes=[
            pltpu.VMEM((L, D), bf16), pltpu.VMEM((G, NB * TP, 128), f32),
            pltpu.VMEM((L, D), f32), pltpu.VMEM((G, TP, 128), f32),
            pltpu.VMEM((2, P, D), bf16), pltpu.VMEM((2, D, P), bf16),
            pltpu.VMEM((7, P, D // 2), bf16), pltpu.VMEM((7, D // 2, P), bf16),
            pltpu.VMEM((D, F), bf16), pltpu.VMEM((D, F), bf16), pltpu.VMEM((F, D), bf16),
            pltpu.VMEM((J, 128), f32), pltpu.VMEM((10, 8, P), f32),
            pltpu.SemaphoreType.DMA((NB + 5 + 2 * NC,)), pltpu.SemaphoreType.DMA((NB + 3,)),
            *[pltpu.VMEM((7, T // 2, D // 2), bf16)] * 4,
            *[pltpu.VMEM((2, 2, T // 2, P), f32)] * 3,
            *[pltpu.VMEM((7, T // 2, P), bf16)] * 3,
        ],
        compiler_params=pltpu.CompilerParams(vmem_limit_bytes=110 * 1024 * 1024,
            flags={'XLA_TPU_EVENLY_DISTRIBUTE_CRITICAL_NODES': True}),
    )(A_x.reshape(L, D), row(A_Lambda_re), row(A_Lambda_im), A_B_re, A_B_im, A_C_re, A_C_im,
      row(A_log_dt), row(A_Dskip), row(B_w_r), B_w_gate, B_w_up, B_w_down)
    return out.reshape(1, L, D)
```

```python
import jax
import jax.numpy as jnp
from jax import lax
import jax.experimental.pallas as pl
import jax.experimental.pallas.tpu as pltpu

L, D, P, F = 2048, 1024, 1024, 3584
T = 256
J = T // 8
NB = L // T
JP = J + 1
TP = 8 * JP
G = P // 128
NC = 4
PC = P // NC
FC = 896
NF = F // FC
f32, bf16 = jnp.float32, jnp.bfloat16
NT = (((1,), (1,)), ((), ()))


def _rb(v):
    return v.astype(bf16).astype(f32)


def _lhs7(a11, a12, a21, a22):
    return (a11 + a22, a21 + a22, a11, a22, a11 + a12, a21 - a11, a12 - a22)


def _rhs7(b11, b12, b21, b22):
    return (b11 + b22, b11, b12 - b22, b21 - b11, b22, b11 + b12, b21 + b22)


def _out4(m):
    return (m[0] + m[3] - m[4] + m[6], m[2] + m[4], m[1] + m[3], m[0] - m[1] + m[2] + m[5])


def _kernel(x_hbm, lre_ref, lim_ref, bre_hbm, bim_hbm, cre_hbm, cim_hbm, ldt_ref, dsk_ref,
            wr_ref, wg_hbm, wu_hbm, wd_hbm, o_hbm,
            xb, xn, ob, yb, bw, cw, bq, cq, wg, wu, wd, rr, st, sem, osem, *rings):
    xq, bu, hq = rings[:4], rings[4:7], rings[7:]

    def cp(src, dst, k):
        return pltpu.make_async_copy(src, dst, sem.at[k])

    x_cp = [cp(x_hbm.at[pl.ds(i * T, T)], xb.at[pl.ds(i * T, T)], i) for i in range(NB)]
    b_cp = [[cp(src.at[pl.ds(k * PC, PC)], bw.at[c, pl.ds(k * PC, PC)], NB + 5 + 2 * k + c)
             for c, src in enumerate((bre_hbm, bim_hbm))] for k in range(NC)]
    c_cp = [cp(cre_hbm, cw.at[0], NB), cp(cim_hbm, cw.at[1], NB + 1)]
    w_cp = [cp(wg_hbm, wg, NB + 2), cp(wu_hbm, wu, NB + 3), cp(wd_hbm, wd, NB + 4)]

    def start(cs):
        for c in cs:
            c.start()

    def wait(cs):
        for c in cs:
            c.wait()

    start(x_cp[:1] + b_cp[0] + x_cp[1:2])

    lre = lre_ref[...].astype(f32).reshape(1, -1)
    lim = lim_ref[...].astype(f32).reshape(1, -1)
    dt = _rb(jnp.exp(ldt_ref[...].astype(f32).reshape(1, -1)))
    ar, ai = dt * lre, dt * lim
    mag = jnp.exp(ar)
    lbr, lbi = mag * jnp.cos(ai), mag * jnp.sin(ai)
    den = lre * lre + lim * lim
    cfr = ((lbr - 1.0) * lre + lbi * lim) / den
    cfi = (lbi * lre - (lbr - 1.0) * lim) / den
    st[0] = jnp.broadcast_to(lbr, (8, P))
    st[1] = jnp.broadcast_to(lbi, (8, P))
    sub = lax.broadcasted_iota(jnp.int32, (8, P), 0)
    for k in range(3):
        n = float(J * (1 << k))
        m = jnp.exp(ar * n)
        keep = sub >= (1 << k)
        st[2 + 2 * k] = jnp.where(keep, jnp.broadcast_to(m * jnp.cos(ai * n), (8, P)), 0.0)
        st[3 + 2 * k] = jnp.where(keep, jnp.broadcast_to(m * jnp.sin(ai * n), (8, P)), 0.0)
    st[8] = jnp.zeros((8, P), f32)
    st[9] = jnp.zeros((8, P), f32)

    dsk = dsk_ref[...].astype(f32).reshape(1, -1)
    dsk1 = dsk + 1.0
    rr[...] = jnp.full((J, 128), -jnp.inf, f32)
    wr = wr_ref[...].astype(f32).reshape(1, -1)

    def lnorm(i):
        for q in range(8):
            rows = pl.ds(i * T + q * J, J)
            x = xb[rows, :].astype(f32)
            mu = jnp.mean(x, axis=-1, keepdims=True)
            c = x - mu
            var = _rb(jnp.mean(c * c, axis=-1, keepdims=True))
            s = _rb(jnp.sqrt(_rb(var + 1e-5)))
            n = _rb(_rb(x - _rb(mu)) * (1.0 / s))
            base = x + n * dsk1
            for g in range(G):
                xn[g, pl.ds(i * TP + q * JP, J), :] = n[:, g * 128:(g + 1) * 128]
            ob[rows, :] = base
            lane = lax.broadcasted_iota(jnp.int32, (J, 128), 1)
            rr[...] = jnp.where(lane == 8 * i + q, _rb(jnp.sum(n * wr, axis=-1, keepdims=True)), rr[...])
        for j in range(0, J, 4):
            for g in range(G // 2):
                def ld(jj, gg):
                    return jnp.concatenate(
                        [xn[gg, pl.ds(i * TP + jj + e, 8, stride=JP), :] for e in (0, 2)], axis=0)
                ops = _lhs7(ld(j, g), ld(j, g + G // 2), ld(j + 1, g), ld(j + 1, g + G // 2))
                for m, v in enumerate(ops):
                    xq[i % 4][m, pl.ds(j * 4, 16), pl.ds(g * 128, 128)] = v.astype(bf16)

    def b_prep(k):
        for r0 in range(k * PC, (k + 1) * PC, 64):
            rows = pl.ds(r0, 64)
            lo, hi = pl.ds(0, D // 2), pl.ds(D // 2, D // 2)
            ops = _rhs7(bw[0, rows, lo].astype(f32), bw[1, rows, lo].astype(f32),
                        bw[0, rows, hi].astype(f32), bw[1, rows, hi].astype(f32))
            for m, v in enumerate(ops):
                if m not in (1, 4):
                    bq[m, rows, :] = v.astype(bf16)

    def c_prep(k):
        kr, ki, nki = 2.0 * cfr, 2.0 * cfi, -2.0 * cfi
        for r0 in range(k * 128, (k + 1) * 128, 16):
            w = []
            for rows in (pl.ds(r0, 16), pl.ds(D // 2 + r0, 16)):
                cr, ci = cw[0, rows, :].astype(f32), cw[1, rows, :].astype(f32)
                w.append((cr * kr - ci * ki, cr * nki - ci * kr))
            for m, v in enumerate(_rhs7(w[0][0], w[1][0], w[0][1], w[1][1])):
                cq[m, pl.ds(r0, 16), :] = v.astype(bf16)

    def mm1(i, k0=0, k1=NC):
        w = pl.ds(k0 * PC, (k1 - k0) * PC)
        rhs = [bw[0, w, pl.ds(0, D // 2)] if m == 1 else bw[1, w, pl.ds(D // 2, D // 2)] if m == 4
               else bq[m, w, :] for m in range(7)]
        c = _out4([lax.dot_general(xq[i % 4][m], rhs[m], NT, preferred_element_type=f32)
                   for m in range(7)])
        for par in range(2):
            for ri in range(2):
                bu[i % 3][ri, par, :, w] = c[2 * par + ri]

    def scan(i, k0=0, k1=NC):
        b, h = bu[i % 3], hq[i % 3]
        for g in range(k0 * PC // 128, k1 * PC // 128):
            ln_ = pl.ds(g * 128, 128)
            a_r, a_i = st[0, :, ln_], st[1, :, ln_]
            c_r, c_i = st[8, :, ln_], st[9, :, ln_]

            def adv(j, sr, si):
                rows = pl.ds((j // 2) * 8, 8)
                return (a_r * sr - a_i * si + b[0, j % 2, rows, ln_],
                        a_r * si + a_i * sr + b[1, j % 2, rows, ln_])

            sr, si = c_r, c_i
            for j in range(J):
                sr, si = adv(j, sr, si)
            for k in range(3):
                pr, pi = st[2 + 2 * k, :, ln_], st[3 + 2 * k, :, ln_]
                qr, qi = pltpu.roll(sr, 1 << k, 0), pltpu.roll(si, 1 << k, 0)
                sr, si = sr + (pr * qr - pi * qi), si + (pr * qi + pi * qr)
            er, ei = pltpu.roll(sr, 1, 0), pltpu.roll(si, 1, 0)
            first = lax.broadcasted_iota(jnp.int32, (8, 128), 0) == 0
            st[8, :, ln_] = jnp.where(first, er, 0.0)
            st[9, :, ln_] = jnp.where(first, ei, 0.0)
            sr, si = jnp.where(first, c_r, er), jnp.where(first, c_i, ei)
            for j in range(0, J, 4):
                o = []
                for jj in range(j, j + 4):
                    sr, si = adv(jj, sr, si)
                    o.append((sr, si))
                lo, hi = _lhs7(*o[0], *o[1]), _lhs7(*o[2], *o[3])
                for m in range(7):
                    h[m, pl.ds(j * 4, 16), ln_] = jnp.concatenate([lo[m], hi[m]], 0).astype(bf16)

    def mm2(i, g0=0, g1=G // 2):
        wrows = pl.ds(g0 * 128, (g1 - g0) * 128)
        c = _out4([lax.dot_general(hq[i % 3][m], cq[m, wrows, :], NT, preferred_element_type=f32)
                   for m in range(7)])
        for j in range(J):
            for half in range(2):
                for g in range(g0, g1):
                    yb[g + half * (G // 2), pl.ds(j, 8, stride=JP), :] = c[2 * (j % 2) + half][
                        (j // 2) * 8:(j // 2 + 1) * 8, (g - g0) * 128:(g - g0 + 1) * 128]
        for q in range(8):
            rows = pl.ds(i * T + q * J, J)
            for half in range(2):
                for g in range(g0 + half * (G // 2), g1 + half * (G // 2)):
                    cols = pl.ds(g * 128, 128)
                    ob[rows, cols] = ob[rows, cols] + yb[g, pl.ds(q * JP, J), :]

    def out_cp(i):
        rows = pl.ds(i * T, T)
        return pltpu.make_async_copy(ob.at[rows], o_hbm.at[rows], osem.at[i])

    def last_cp(q):
        rows = pl.ds((NB - 1) * T, T)
        return [pltpu.make_async_copy(ob.at[rows, cols], o_hbm.at[rows, cols], osem.at[NB - 1 + 2 * q + e])
                for e, cols in enumerate((pl.ds(q * 256, 256), pl.ds(D // 2 + q * 256, 256)))]

    def get_row(ref, idx):
        return jnp.concatenate([ref[g, pl.ds(idx + idx // J, 1), :] for g in range(G)], axis=1)

    wait(x_cp[:1])
    start(b_cp[1])
    lnorm(0)
    for k in range(NC):
        wait(b_cp[k] + (x_cp[1:2] if k == 0 else x_cp[2:3] if k == 2 else []))
        start((x_cp[2:3] + b_cp[2], x_cp[3:4] + b_cp[3], c_cp, x_cp[4:])[k])
        b_prep(k)
        mm1(0, k, k + 1)
        if k in (0, 2):
            lnorm(1 + k // 2)
        mm1(1, k, k + 1)
        if k > 0:
            scan(0, k - 1, k)
            scan(1, k - 1, k)
    wait(c_cp)
    start(w_cp)
    for k in range(NC):
        mm1(2, k, k + 1)
        if k % 2 == 0:
            c_prep(k // 2)
        if k < 2:
            scan(k, NC - 1, NC)
    wait(x_cp[3:4])
    mm2(0, 0, 2)
    c_prep(2)
    c_prep(3)
    lnorm(3)
    for i in range(NB - 4):
        wait(x_cp[i + 4:i + 5])
        lnorm(i + 4)
        mm2(i, 2 if i == 0 else 0)
        scan(i + 2)
        mm1(i + 3)
    wait(w_cp)
    r = rr[...]
    lane = lax.broadcasted_iota(jnp.int32, (J, 128), 1)
    ti = jnp.where(lane < L // J, lane * J + lax.broadcasted_iota(jnp.int32, (J, 128), 0), L)

    def red(op, v):
        return op(op(v, axis=0, keepdims=True), axis=1, keepdims=True)

    m0 = red(jnp.max, r)
    i0v = red(jnp.min, jnp.where(r == m0, ti, L))
    r2 = jnp.where(ti == i0v, -jnp.inf, r)
    m1 = red(jnp.max, r2)
    i1v = red(jnp.min, jnp.where((r2 == m1) & (ti != i0v), ti, L))
    i0 = jnp.clip(i0v[0, 0], 0, L - 1)
    i1 = jnp.clip(i1v[0, 0], 0, L - 1)

    s8 = lax.broadcasted_iota(jnp.int32, (16, D), 0)
    xs = jnp.where(s8 == 0, get_row(xn, i0), jnp.where(s8 == 1, get_row(xn, i1), 0.0)).astype(bf16)
    mm2(NB - 4)
    scan(NB - 2)
    mm1(NB - 1)
    acc = jnp.zeros((16, D), f32)
    for c in range(NF):
        cols = pl.ds(c * FC, FC)
        gt = _rb(jnp.dot(xs, wg[:, cols], preferred_element_type=f32))
        gt = _rb(gt * _rb(jax.nn.sigmoid(gt)))
        up = _rb(jnp.dot(xs, wu[:, cols], preferred_element_type=f32))
        acc = acc + jnp.dot((gt * up).astype(bf16), wd[cols, :], preferred_element_type=f32)
    yf = _rb(acc)
    for k, (idx, m) in enumerate(((i0, m0), (i1, m1))):
        row = pl.ds(idx, 1)
        n = get_row(xn, idx)
        upd = _rb(yf[k:k + 1, :] * _rb(jax.nn.sigmoid(m)))
        dl = _rb(n + upd) - n
        ob[row, :] = ob[row, :] + dl
    start([out_cp(i) for i in range(NB - 3)])
    mm2(NB - 3)
    scan(NB - 1)
    out_cp(0).wait()
    out_cp(NB - 3).start()
    mm2(NB - 2)
    out_cp(1).wait()
    out_cp(NB - 2).start()
    for q in range(2):
        mm2(NB - 1, 2 * q, 2 * q + 2)
        start(last_cp(q))
    wait([out_cp(i) for i in range(2, NB - 1)] + last_cp(0) + last_cp(1))


@jax.jit
def pallas_parallel_sum__ssm_conv_s5__moe_arch_mod__prompt_kernel(
    A_x, A_Lambda_re, A_Lambda_im, A_B_re, A_B_im, A_C_re, A_C_im, A_log_dt, A_Dskip,
    B_x, B_w_r, B_w_gate, B_w_up, B_w_down,
):
    hbm = pl.BlockSpec(memory_space=pl.ANY)
    vm = pl.BlockSpec(memory_space=pltpu.VMEM)
    row = lambda v: v
    out = pl.pallas_call(
        _kernel,
        out_shape=jax.ShapeDtypeStruct((L, D), f32),
        in_specs=[hbm, vm, vm, hbm, hbm, hbm, hbm, vm, vm, vm, hbm, hbm, hbm],
        out_specs=hbm,
        scratch_shapes=[
            pltpu.VMEM((L, D), bf16), pltpu.VMEM((G, NB * TP, 128), f32),
            pltpu.VMEM((L, D), f32), pltpu.VMEM((G, TP, 128), f32),
            pltpu.VMEM((2, P, D), bf16), pltpu.VMEM((2, D, P), bf16),
            pltpu.VMEM((7, P, D // 2), bf16), pltpu.VMEM((7, D // 2, P), bf16),
            pltpu.VMEM((D, F), bf16), pltpu.VMEM((D, F), bf16), pltpu.VMEM((F, D), bf16),
            pltpu.VMEM((J, 128), f32), pltpu.VMEM((10, 8, P), f32),
            pltpu.SemaphoreType.DMA((NB + 5 + 2 * NC,)), pltpu.SemaphoreType.DMA((NB + 3,)),
            *[pltpu.VMEM((7, T // 2, D // 2), bf16)] * 4,
            *[pltpu.VMEM((2, 2, T // 2, P), f32)] * 3,
            *[pltpu.VMEM((7, T // 2, P), bf16)] * 3,
        ],
        compiler_params=pltpu.CompilerParams(vmem_limit_bytes=110 * 1024 * 1024,
            flags={'XLA_TPU_EVENLY_DISTRIBUTE_CRITICAL_NODES': True}),
    )(A_x.reshape(L, D), row(A_Lambda_re), row(A_Lambda_im), A_B_re, A_B_im, A_C_re, A_C_im,
      row(A_log_dt), row(A_Dskip), row(B_w_r), B_w_gate, B_w_up, B_w_down)
    return out.reshape(1, L, D)
```

```python
import jax
import jax.numpy as jnp
from jax import lax
import jax.experimental.pallas as pl
import jax.experimental.pallas.tpu as pltpu

L, D, P, F = 2048, 1024, 1024, 3584
T = 256
J = T // 8
NB = L // T
JP = J + 1
TP = 8 * JP
G = P // 128
NC = 4
PC = P // NC
FC = 896
NF = F // FC
f32, bf16 = jnp.float32, jnp.bfloat16
NT = (((1,), (1,)), ((), ()))


def _rb(v):
    return v.astype(bf16).astype(f32)


def _lhs7(a11, a12, a21, a22):
    return (a11 + a22, a21 + a22, a11, a22, a11 + a12, a21 - a11, a12 - a22)


def _rhs7(b11, b12, b21, b22):
    return (b11 + b22, b11, b12 - b22, b21 - b11, b22, b11 + b12, b21 + b22)


def _out4(m):
    return (m[0] + m[3] - m[4] + m[6], m[2] + m[4], m[1] + m[3], m[0] - m[1] + m[2] + m[5])


def _kernel(x_hbm, lre_ref, lim_ref, bre_hbm, bim_hbm, cre_hbm, cim_hbm, ldt_ref, dsk_ref,
            wr_ref, wg_hbm, wu_hbm, wd_hbm, o_hbm,
            xb, xn, ob, yb, bw, cw, bq, cq, wg, wu, wd, rr, st, sem, osem, *rings):
    xq, bu, hq = rings[:4], rings[4:7], rings[7:]

    def cp(src, dst, k):
        return pltpu.make_async_copy(src, dst, sem.at[k])

    x_cp = [cp(x_hbm.at[pl.ds(i * T, T)], xb.at[pl.ds(i * T, T)], i) for i in range(NB)]
    b_cp = [[cp(src.at[pl.ds(k * PC, PC)], bw.at[c, pl.ds(k * PC, PC)], NB + 5 + 2 * k + c)
             for c, src in enumerate((bre_hbm, bim_hbm))] for k in range(NC)]
    c_cp = [cp(cre_hbm, cw.at[0], NB), cp(cim_hbm, cw.at[1], NB + 1)]
    w_cp = [cp(wg_hbm, wg, NB + 2), cp(wu_hbm, wu, NB + 3), cp(wd_hbm, wd, NB + 4)]

    def start(cs):
        for c in cs:
            c.start()

    def wait(cs):
        for c in cs:
            c.wait()

    start(x_cp[:1] + b_cp[0] + x_cp[1:2])

    lre = lre_ref[...].astype(f32).reshape(1, -1)
    lim = lim_ref[...].astype(f32).reshape(1, -1)
    dt = _rb(jnp.exp(ldt_ref[...].astype(f32).reshape(1, -1)))
    ar, ai = dt * lre, dt * lim
    mag = jnp.exp(ar)
    lbr, lbi = mag * jnp.cos(ai), mag * jnp.sin(ai)
    den = lre * lre + lim * lim
    cfr = ((lbr - 1.0) * lre + lbi * lim) / den
    cfi = (lbi * lre - (lbr - 1.0) * lim) / den
    st[0] = jnp.broadcast_to(lbr, (8, P))
    st[1] = jnp.broadcast_to(lbi, (8, P))
    sub = lax.broadcasted_iota(jnp.int32, (8, P), 0)
    for k in range(3):
        n = float(J * (1 << k))
        m = jnp.exp(ar * n)
        keep = sub >= (1 << k)
        st[2 + 2 * k] = jnp.where(keep, jnp.broadcast_to(m * jnp.cos(ai * n), (8, P)), 0.0)
        st[3 + 2 * k] = jnp.where(keep, jnp.broadcast_to(m * jnp.sin(ai * n), (8, P)), 0.0)
    st[8] = jnp.zeros((8, P), f32)
    st[9] = jnp.zeros((8, P), f32)

    dsk = dsk_ref[...].astype(f32).reshape(1, -1)
    dsk1 = dsk + 1.0
    rr[...] = jnp.full((J, 128), -jnp.inf, f32)
    wr = wr_ref[...].astype(f32).reshape(1, -1)

    def lnorm(i):
        for q in range(8):
            rows = pl.ds(i * T + q * J, J)
            x = xb[rows, :].astype(f32)
            mu = jnp.mean(x, axis=-1, keepdims=True)
            c = x - mu
            var = _rb(jnp.mean(c * c, axis=-1, keepdims=True))
            s = _rb(jnp.sqrt(_rb(var + 1e-5)))
            n = _rb(_rb(x - _rb(mu)) * (1.0 / s))
            base = x + n * dsk1
            for g in range(G):
                xn[g, pl.ds(i * TP + q * JP, J), :] = n[:, g * 128:(g + 1) * 128]
            ob[rows, :] = base
            lane = lax.broadcasted_iota(jnp.int32, (J, 128), 1)
            rr[...] = jnp.where(lane == 8 * i + q, _rb(jnp.sum(n * wr, axis=-1, keepdims=True)), rr[...])
        for j in range(0, J, 4):
            for g in range(G // 2):
                def ld(jj, gg):
                    return jnp.concatenate(
                        [xn[gg, pl.ds(i * TP + jj + e, 8, stride=JP), :] for e in (0, 2)], axis=0)
                ops = _lhs7(ld(j, g), ld(j, g + G // 2), ld(j + 1, g), ld(j + 1, g + G // 2))
                for m, v in enumerate(ops):
                    xq[i % 4][m, pl.ds(j * 4, 16), pl.ds(g * 128, 128)] = v.astype(bf16)

    def b_prep(k):
        for r0 in range(k * PC, (k + 1) * PC, 64):
            rows = pl.ds(r0, 64)
            lo, hi = pl.ds(0, D // 2), pl.ds(D // 2, D // 2)
            ops = _rhs7(bw[0, rows, lo].astype(f32), bw[1, rows, lo].astype(f32),
                        bw[0, rows, hi].astype(f32), bw[1, rows, hi].astype(f32))
            for m, v in enumerate(ops):
                if m not in (1, 4):
                    bq[m, rows, :] = v.astype(bf16)

    def c_prep(k):
        kr, ki, nki = 2.0 * cfr, 2.0 * cfi, -2.0 * cfi
        for r0 in range(k * 128, (k + 1) * 128, 16):
            w = []
            for rows in (pl.ds(r0, 16), pl.ds(D // 2 + r0, 16)):
                cr, ci = cw[0, rows, :].astype(f32), cw[1, rows, :].astype(f32)
                w.append((cr * kr - ci * ki, cr * nki - ci * kr))
            for m, v in enumerate(_rhs7(w[0][0], w[1][0], w[0][1], w[1][1])):
                cq[m, pl.ds(r0, 16), :] = v.astype(bf16)

    def mm1(i, k0=0, k1=NC):
        w = pl.ds(k0 * PC, (k1 - k0) * PC)
        rhs = [bw[0, w, pl.ds(0, D // 2)] if m == 1 else bw[1, w, pl.ds(D // 2, D // 2)] if m == 4
               else bq[m, w, :] for m in range(7)]
        c = _out4([lax.dot_general(xq[i % 4][m], rhs[m], NT, preferred_element_type=f32)
                   for m in range(7)])
        for par in range(2):
            for ri in range(2):
                bu[i % 3][ri, par, :, w] = c[2 * par + ri]

    def scan(i, k0=0, k1=NC):
        b, h = bu[i % 3], hq[i % 3]
        for g in range(k0 * PC // 128, k1 * PC // 128):
            ln_ = pl.ds(g * 128, 128)
            a_r, a_i = st[0, :, ln_], st[1, :, ln_]
            c_r, c_i = st[8, :, ln_], st[9, :, ln_]

            def adv(j, sr, si):
                rows = pl.ds((j // 2) * 8, 8)
                return (a_r * sr - a_i * si + b[0, j % 2, rows, ln_],
                        a_r * si + a_i * sr + b[1, j % 2, rows, ln_])

            sr, si = c_r, c_i
            for j in range(J):
                sr, si = adv(j, sr, si)
            for k in range(3):
                pr, pi = st[2 + 2 * k, :, ln_], st[3 + 2 * k, :, ln_]
                qr, qi = pltpu.roll(sr, 1 << k, 0), pltpu.roll(si, 1 << k, 0)
                sr, si = sr + (pr * qr - pi * qi), si + (pr * qi + pi * qr)
            er, ei = pltpu.roll(sr, 1, 0), pltpu.roll(si, 1, 0)
            first = lax.broadcasted_iota(jnp.int32, (8, 128), 0) == 0
            st[8, :, ln_] = jnp.where(first, er, 0.0)
            st[9, :, ln_] = jnp.where(first, ei, 0.0)
            sr, si = jnp.where(first, c_r, er), jnp.where(first, c_i, ei)
            for j in range(0, J, 4):
                o = []
                for jj in range(j, j + 4):
                    sr, si = adv(jj, sr, si)
                    o.append((sr, si))
                lo, hi = _lhs7(*o[0], *o[1]), _lhs7(*o[2], *o[3])
                for m in range(7):
                    h[m, pl.ds(j * 4, 16), ln_] = jnp.concatenate([lo[m], hi[m]], 0).astype(bf16)

    def mm2(i, g0=0, g1=G // 2):
        wrows = pl.ds(g0 * 128, (g1 - g0) * 128)
        c = _out4([lax.dot_general(hq[i % 3][m], cq[m, wrows, :], NT, preferred_element_type=f32)
                   for m in range(7)])
        for j in range(J):
            for half in range(2):
                for g in range(g0, g1):
                    yb[g + half * (G // 2), pl.ds(j, 8, stride=JP), :] = c[2 * (j % 2) + half][
                        (j // 2) * 8:(j // 2 + 1) * 8, (g - g0) * 128:(g - g0 + 1) * 128]
        for q in range(8):
            rows = pl.ds(i * T + q * J, J)
            for half in range(2):
                for g in range(g0 + half * (G // 2), g1 + half * (G // 2)):
                    cols = pl.ds(g * 128, 128)
                    ob[rows, cols] = ob[rows, cols] + yb[g, pl.ds(q * JP, J), :]

    def out_cp(i):
        rows = pl.ds(i * T, T)
        return pltpu.make_async_copy(ob.at[rows], o_hbm.at[rows], osem.at[i])

    def last_cp(q):
        rows = pl.ds((NB - 1) * T, T)
        return [pltpu.make_async_copy(ob.at[rows, cols], o_hbm.at[rows, cols], osem.at[NB - 1 + 2 * q + e])
                for e, cols in enumerate((pl.ds(q * 256, 256), pl.ds(D // 2 + q * 256, 256)))]

    def get_row(ref, idx):
        return jnp.concatenate([ref[g, pl.ds(idx + idx // J, 1), :] for g in range(G)], axis=1)

    wait(x_cp[:1])
    start(b_cp[1])
    lnorm(0)
    for k in range(NC):
        wait(b_cp[k] + (x_cp[1:2] if k == 0 else x_cp[2:3] if k == 2 else []))
        start((x_cp[2:3] + b_cp[2], x_cp[3:4] + b_cp[3], c_cp, x_cp[4:])[k])
        b_prep(k)
        mm1(0, k, k + 1)
        if k in (0, 2):
            lnorm(1 + k // 2)
        mm1(1, k, k + 1)
        if k > 0:
            scan(0, k - 1, k)
            scan(1, k - 1, k)
    wait(c_cp)
    start(w_cp)
    for k in range(NC):
        mm1(2, k, k + 1)
        if k % 2 == 0:
            c_prep(k // 2)
        if k < 2:
            scan(k, NC - 1, NC)
    wait(x_cp[3:4])
    mm2(0, 0, 2)
    c_prep(2)
    c_prep(3)
    lnorm(3)
    for i in range(NB - 4):
        wait(x_cp[i + 4:i + 5])
        lnorm(i + 4)
        mm2(i, 2 if i == 0 else 0)
        scan(i + 2)
        mm1(i + 3)
    wait(w_cp)
    r = rr[...]
    lane = lax.broadcasted_iota(jnp.int32, (J, 128), 1)
    ti = jnp.where(lane < L // J, lane * J + lax.broadcasted_iota(jnp.int32, (J, 128), 0), L)

    def red(op, v):
        return op(op(v, axis=0, keepdims=True), axis=1, keepdims=True)

    m0 = red(jnp.max, r)
    i0v = red(jnp.min, jnp.where(r == m0, ti, L))
    r2 = jnp.where(ti == i0v, -jnp.inf, r)
    m1 = red(jnp.max, r2)
    i1v = red(jnp.min, jnp.where((r2 == m1) & (ti != i0v), ti, L))
    i0 = jnp.clip(i0v[0, 0], 0, L - 1)
    i1 = jnp.clip(i1v[0, 0], 0, L - 1)

    s8 = lax.broadcasted_iota(jnp.int32, (16, D), 0)
    xs = jnp.where(s8 == 0, get_row(xn, i0), jnp.where(s8 == 1, get_row(xn, i1), 0.0)).astype(bf16)
    mm2(NB - 4)
    scan(NB - 2)
    mm1(NB - 1)
    acc = jnp.zeros((16, D), f32)
    for c in range(NF):
        cols = pl.ds(c * FC, FC)
        gt = _rb(jnp.dot(xs, wg[:, cols], preferred_element_type=f32))
        gt = _rb(gt * _rb(jax.nn.sigmoid(gt)))
        up = _rb(jnp.dot(xs, wu[:, cols], preferred_element_type=f32))
        acc = acc + jnp.dot((gt * up).astype(bf16), wd[cols, :], preferred_element_type=f32)
    yf = _rb(acc)
    for k, (idx, m) in enumerate(((i0, m0), (i1, m1))):
        row = pl.ds(idx, 1)
        n = get_row(xn, idx)
        upd = _rb(yf[k:k + 1, :] * _rb(jax.nn.sigmoid(m)))
        dl = _rb(n + upd) - n
        ob[row, :] = ob[row, :] + dl
    start([out_cp(i) for i in range(NB - 3)])
    mm2(NB - 3)
    scan(NB - 1, 0, NC // 2)
    out_cp(0).wait()
    out_cp(NB - 3).start()
    mm2(NB - 2)
    scan(NB - 1, NC // 2, NC)
    out_cp(1).wait()
    out_cp(NB - 2).start()
    out_cp(2).wait()
    for q in range(2):
        mm2(NB - 1, 2 * q, 2 * q + 2)
        start(last_cp(q))
    wait([out_cp(i) for i in range(3, NB - 1)] + last_cp(0) + last_cp(1))


@jax.jit
def pallas_parallel_sum__ssm_conv_s5__moe_arch_mod__prompt_kernel(
    A_x, A_Lambda_re, A_Lambda_im, A_B_re, A_B_im, A_C_re, A_C_im, A_log_dt, A_Dskip,
    B_x, B_w_r, B_w_gate, B_w_up, B_w_down,
):
    hbm = pl.BlockSpec(memory_space=pl.ANY)
    vm = pl.BlockSpec(memory_space=pltpu.VMEM)
    row = lambda v: v
    out = pl.pallas_call(
        _kernel,
        out_shape=jax.ShapeDtypeStruct((L, D), f32),
        in_specs=[hbm, vm, vm, hbm, hbm, hbm, hbm, vm, vm, vm, hbm, hbm, hbm],
        out_specs=hbm,
        scratch_shapes=[
            pltpu.VMEM((L, D), bf16), pltpu.VMEM((G, NB * TP, 128), f32),
            pltpu.VMEM((L, D), f32), pltpu.VMEM((G, TP, 128), f32),
            pltpu.VMEM((2, P, D), bf16), pltpu.VMEM((2, D, P), bf16),
            pltpu.VMEM((7, P, D // 2), bf16), pltpu.VMEM((7, D // 2, P), bf16),
            pltpu.VMEM((D, F), bf16), pltpu.VMEM((D, F), bf16), pltpu.VMEM((F, D), bf16),
            pltpu.VMEM((J, 128), f32), pltpu.VMEM((10, 8, P), f32),
            pltpu.SemaphoreType.DMA((NB + 5 + 2 * NC,)), pltpu.SemaphoreType.DMA((NB + 3,)),
            *[pltpu.VMEM((7, T // 2, D // 2), bf16)] * 4,
            *[pltpu.VMEM((2, 2, T // 2, P), f32)] * 3,
            *[pltpu.VMEM((7, T // 2, P), bf16)] * 3,
        ],
        compiler_params=pltpu.CompilerParams(vmem_limit_bytes=110 * 1024 * 1024,
            flags={'XLA_TPU_EVENLY_DISTRIBUTE_CRITICAL_NODES': True}),
    )(A_x.reshape(L, D), row(A_Lambda_re), row(A_Lambda_im), A_B_re, A_B_im, A_C_re, A_C_im,
      row(A_log_dt), row(A_Dskip), row(B_w_r), B_w_gate, B_w_up, B_w_down)
    return out.reshape(1, L, D)
```

```python
import jax
import jax.numpy as jnp
from jax import lax
import jax.experimental.pallas as pl
import jax.experimental.pallas.tpu as pltpu

L, D, P, F = 2048, 1024, 1024, 3584
T = 256
J = T // 8
NB = L // T
JP = J + 1
TP = 8 * JP
G = P // 128
NC = 4
PC = P // NC
FC = 896
NF = F // FC
f32, bf16 = jnp.float32, jnp.bfloat16
NT = (((1,), (1,)), ((), ()))


def _rb(v):
    return v.astype(bf16).astype(f32)


def _lhs7(a11, a12, a21, a22):
    return (a11 + a22, a21 + a22, a11, a22, a11 + a12, a21 - a11, a12 - a22)


def _rhs7(b11, b12, b21, b22):
    return (b11 + b22, b11, b12 - b22, b21 - b11, b22, b11 + b12, b21 + b22)


def _out4(m):
    return (m[0] + m[3] - m[4] + m[6], m[2] + m[4], m[1] + m[3], m[0] - m[1] + m[2] + m[5])


def _kernel(x_hbm, lre_ref, lim_ref, bre_hbm, bim_hbm, cre_hbm, cim_hbm, ldt_ref, dsk_ref,
            wr_ref, wg_hbm, wu_hbm, wd_hbm, o_hbm,
            xb, xn, ob, yb, bw, cw, bq, cq, wg, wu, wd, rr, st, sem, osem, *rings):
    xq, bu, hq = rings[:4], rings[4:7], rings[7:]

    def cp(src, dst, k):
        return pltpu.make_async_copy(src, dst, sem.at[k])

    x_cp = [cp(x_hbm.at[pl.ds(i * T, T)], xb.at[pl.ds(i * T, T)], i) for i in range(NB)]
    b_cp = [[cp(src.at[pl.ds(k * PC, PC)], bw.at[c, pl.ds(k * PC, PC)], NB + 5 + 2 * k + c)
             for c, src in enumerate((bre_hbm, bim_hbm))] for k in range(NC)]
    c_cp = [cp(cre_hbm, cw.at[0], NB), cp(cim_hbm, cw.at[1], NB + 1)]
    w_cp = [cp(wg_hbm, wg, NB + 2), cp(wu_hbm, wu, NB + 3), cp(wd_hbm, wd, NB + 4)]

    def start(cs):
        for c in cs:
            c.start()

    def wait(cs):
        for c in cs:
            c.wait()

    start(x_cp[:1] + b_cp[0] + x_cp[1:2])

    lre = lre_ref[...].astype(f32).reshape(1, -1)
    lim = lim_ref[...].astype(f32).reshape(1, -1)
    dt = _rb(jnp.exp(ldt_ref[...].astype(f32).reshape(1, -1)))
    ar, ai = dt * lre, dt * lim
    mag = jnp.exp(ar)
    lbr, lbi = mag * jnp.cos(ai), mag * jnp.sin(ai)
    nr, ni = lbr - 1.0, lbi
    wide = jnp.abs(lre) >= jnp.abs(lim)
    big, small = jnp.where(wide, lre, lim), jnp.where(wide, lim, lre)
    rat = small / big
    den = big + small * rat
    cfr = jnp.where(wide, nr + ni * rat, nr * rat + ni) / den
    cfi = jnp.where(wide, ni - nr * rat, ni * rat - nr) / den
    st[0] = jnp.broadcast_to(lbr, (8, P))
    st[1] = jnp.broadcast_to(lbi, (8, P))
    sub = lax.broadcasted_iota(jnp.int32, (8, P), 0)
    for k in range(3):
        n = float(J * (1 << k))
        m = jnp.exp(ar * n)
        keep = sub >= (1 << k)
        st[2 + 2 * k] = jnp.where(keep, jnp.broadcast_to(m * jnp.cos(ai * n), (8, P)), 0.0)
        st[3 + 2 * k] = jnp.where(keep, jnp.broadcast_to(m * jnp.sin(ai * n), (8, P)), 0.0)
    st[8] = jnp.zeros((8, P), f32)
    st[9] = jnp.zeros((8, P), f32)

    dsk = dsk_ref[...].astype(f32).reshape(1, -1)
    dsk1 = dsk + 1.0
    rr[...] = jnp.full((J, 128), -jnp.inf, f32)
    wr = wr_ref[...].astype(f32).reshape(1, -1)

    def lnorm(i):
        for q in range(8):
            rows = pl.ds(i * T + q * J, J)
            x = xb[rows, :].astype(f32)
            mu = jnp.mean(x, axis=-1, keepdims=True)
            c = x - mu
            var = _rb(jnp.mean(c * c, axis=-1, keepdims=True))
            s = _rb(jnp.sqrt(_rb(var + 1e-5)))
            n = _rb(_rb(x - _rb(mu)) * (1.0 / s))
            base = x + n * dsk1
            for g in range(G):
                xn[g, pl.ds(i * TP + q * JP, J), :] = n[:, g * 128:(g + 1) * 128]
            ob[rows, :] = base
            lane = lax.broadcasted_iota(jnp.int32, (J, 128), 1)
            rr[...] = jnp.where(lane == 8 * i + q, _rb(jnp.sum(n * wr, axis=-1, keepdims=True)), rr[...])
        for j in range(0, J, 4):
            for g in range(G // 2):
                def ld(jj, gg):
                    return jnp.concatenate(
                        [xn[gg, pl.ds(i * TP + jj + e, 8, stride=JP), :] for e in (0, 2)], axis=0)
                ops = _lhs7(ld(j, g), ld(j, g + G // 2), ld(j + 1, g), ld(j + 1, g + G // 2))
                for m, v in enumerate(ops):
                    xq[i % 4][m, pl.ds(j * 4, 16), pl.ds(g * 128, 128)] = v.astype(bf16)

    def b_prep(k):
        for r0 in range(k * PC, (k + 1) * PC, 64):
            rows = pl.ds(r0, 64)
            lo, hi = pl.ds(0, D // 2), pl.ds(D // 2, D // 2)
            ops = _rhs7(bw[0, rows, lo].astype(f32), bw[1, rows, lo].astype(f32),
                        bw[0, rows, hi].astype(f32), bw[1, rows, hi].astype(f32))
            for m, v in enumerate(ops):
                if m not in (1, 4):
                    bq[m, rows, :] = v.astype(bf16)

    def c_prep(k):
        kr, ki, nki = 2.0 * cfr, 2.0 * cfi, -2.0 * cfi
        for r0 in range(k * 128, (k + 1) * 128, 16):
            w = []
            for rows in (pl.ds(r0, 16), pl.ds(D // 2 + r0, 16)):
                cr, ci = cw[0, rows, :].astype(f32), cw[1, rows, :].astype(f32)
                w.append((cr * kr - ci * ki, cr * nki - ci * kr))
            for m, v in enumerate(_rhs7(w[0][0], w[1][0], w[0][1], w[1][1])):
                cq[m, pl.ds(r0, 16), :] = v.astype(bf16)

    def mm1(i, k0=0, k1=NC):
        w = pl.ds(k0 * PC, (k1 - k0) * PC)
        rhs = [bw[0, w, pl.ds(0, D // 2)] if m == 1 else bw[1, w, pl.ds(D // 2, D // 2)] if m == 4
               else bq[m, w, :] for m in range(7)]
        c = _out4([lax.dot_general(xq[i % 4][m], rhs[m], NT, preferred_element_type=f32)
                   for m in range(7)])
        for par in range(2):
            for ri in range(2):
                bu[i % 3][ri, par, :, w] = c[2 * par + ri]

    def scan(i, k0=0, k1=NC):
        b, h = bu[i % 3], hq[i % 3]
        for g in range(k0 * PC // 128, k1 * PC // 128):
            ln_ = pl.ds(g * 128, 128)
            a_r, a_i = st[0, :, ln_], st[1, :, ln_]
            c_r, c_i = st[8, :, ln_], st[9, :, ln_]

            def adv(j, sr, si):
                rows = pl.ds((j // 2) * 8, 8)
                return (a_r * sr - a_i * si + b[0, j % 2, rows, ln_],
                        a_r * si + a_i * sr + b[1, j % 2, rows, ln_])

            sr, si = c_r, c_i
            for j in range(J):
                sr, si = adv(j, sr, si)
            for k in range(3):
                pr, pi = st[2 + 2 * k, :, ln_], st[3 + 2 * k, :, ln_]
                qr, qi = pltpu.roll(sr, 1 << k, 0), pltpu.roll(si, 1 << k, 0)
                sr, si = sr + (pr * qr - pi * qi), si + (pr * qi + pi * qr)
            er, ei = pltpu.roll(sr, 1, 0), pltpu.roll(si, 1, 0)
            first = lax.broadcasted_iota(jnp.int32, (8, 128), 0) == 0
            st[8, :, ln_] = jnp.where(first, er, 0.0)
            st[9, :, ln_] = jnp.where(first, ei, 0.0)
            sr, si = jnp.where(first, c_r, er), jnp.where(first, c_i, ei)
            for j in range(0, J, 4):
                o = []
                for jj in range(j, j + 4):
                    sr, si = adv(jj, sr, si)
                    o.append((sr, si))
                lo, hi = _lhs7(*o[0], *o[1]), _lhs7(*o[2], *o[3])
                for m in range(7):
                    h[m, pl.ds(j * 4, 16), ln_] = jnp.concatenate([lo[m], hi[m]], 0).astype(bf16)

    def mm2(i, g0=0, g1=G // 2):
        wrows = pl.ds(g0 * 128, (g1 - g0) * 128)
        c = _out4([lax.dot_general(hq[i % 3][m], cq[m, wrows, :], NT, preferred_element_type=f32)
                   for m in range(7)])
        for j in range(J):
            for half in range(2):
                for g in range(g0, g1):
                    yb[g + half * (G // 2), pl.ds(j, 8, stride=JP), :] = c[2 * (j % 2) + half][
                        (j // 2) * 8:(j // 2 + 1) * 8, (g - g0) * 128:(g - g0 + 1) * 128]
        for q in range(8):
            rows = pl.ds(i * T + q * J, J)
            for half in range(2):
                for g in range(g0 + half * (G // 2), g1 + half * (G // 2)):
                    cols = pl.ds(g * 128, 128)
                    ob[rows, cols] = ob[rows, cols] + yb[g, pl.ds(q * JP, J), :]

    def out_cp(i):
        rows = pl.ds(i * T, T)
        return pltpu.make_async_copy(ob.at[rows], o_hbm.at[rows], osem.at[i])

    def last_cp(q):
        rows = pl.ds((NB - 1) * T, T)
        return [pltpu.make_async_copy(ob.at[rows, cols], o_hbm.at[rows, cols], osem.at[NB - 1 + 2 * q + e])
                for e, cols in enumerate((pl.ds(q * 128, 128), pl.ds(D // 2 + q * 128, 128)))]

    def get_row(ref, idx):
        return jnp.concatenate([ref[g, pl.ds(idx + idx // J, 1), :] for g in range(G)], axis=1)

    wait(x_cp[:1])
    start(b_cp[1])
    lnorm(0)
    for k in range(NC):
        wait(b_cp[k] + (x_cp[1:2] if k == 0 else x_cp[2:3] if k == 2 else []))
        start((x_cp[2:3] + b_cp[2], x_cp[3:4] + b_cp[3], c_cp, x_cp[4:])[k])
        b_prep(k)
        mm1(0, k, k + 1)
        if k in (0, 2):
            lnorm(1 + k // 2)
        mm1(1, k, k + 1)
        if k > 0:
            scan(0, k - 1, k)
            scan(1, k - 1, k)
    wait(c_cp)
    start(w_cp)
    for k in range(NC):
        mm1(2, k, k + 1)
        if k % 2 == 0:
            c_prep(k // 2)
        if k < 2:
            scan(k, NC - 1, NC)
    wait(x_cp[3:4])
    mm2(0, 0, 2)
    c_prep(2)
    c_prep(3)
    lnorm(3)
    for i in range(NB - 4):
        wait(x_cp[i + 4:i + 5])
        lnorm(i + 4)
        mm2(i, 2 if i == 0 else 0)
        scan(i + 2)
        mm1(i + 3)
    wait(w_cp)
    r = rr[...]
    lane = lax.broadcasted_iota(jnp.int32, (J, 128), 1)
    ti = jnp.where(lane < L // J, lane * J + lax.broadcasted_iota(jnp.int32, (J, 128), 0), L)

    def red(op, v):
        return op(op(v, axis=0, keepdims=True), axis=1, keepdims=True)

    m0 = red(jnp.max, r)
    i0v = red(jnp.min, jnp.where(r == m0, ti, L))
    r2 = jnp.where(ti == i0v, -jnp.inf, r)
    m1 = red(jnp.max, r2)
    i1v = red(jnp.min, jnp.where((r2 == m1) & (ti != i0v), ti, L))
    i0 = jnp.clip(i0v[0, 0], 0, L - 1)
    i1 = jnp.clip(i1v[0, 0], 0, L - 1)

    s8 = lax.broadcasted_iota(jnp.int32, (16, D), 0)
    xs = jnp.where(s8 == 0, get_row(xn, i0), jnp.where(s8 == 1, get_row(xn, i1), 0.0)).astype(bf16)
    mm2(NB - 4)
    scan(NB - 2)
    mm1(NB - 1)
    acc = jnp.zeros((16, D), f32)
    for c in range(NF):
        cols = pl.ds(c * FC, FC)
        gt = _rb(jnp.dot(xs, wg[:, cols], preferred_element_type=f32))
        gt = _rb(gt * _rb(jax.nn.sigmoid(gt)))
        up = _rb(jnp.dot(xs, wu[:, cols], preferred_element_type=f32))
        acc = acc + jnp.dot((gt * up).astype(bf16), wd[cols, :], preferred_element_type=f32)
    yf = _rb(acc)
    for k, (idx, m) in enumerate(((i0, m0), (i1, m1))):
        row = pl.ds(idx, 1)
        n = get_row(xn, idx)
        upd = _rb(yf[k:k + 1, :] * _rb(jax.nn.sigmoid(m)))
        dl = _rb(n + upd) - n
        ob[row, :] = ob[row, :] + dl
    start([out_cp(i) for i in range(NB - 3)])
    mm2(NB - 3)
    scan(NB - 1, 0, NC // 2)
    out_cp(0).wait()
    out_cp(NB - 3).start()
    mm2(NB - 2)
    scan(NB - 1, NC // 2, NC)
    out_cp(1).wait()
    out_cp(NB - 2).start()
    out_cp(2).wait()
    for q in range(4):
        mm2(NB - 1, q, q + 1)
        start(last_cp(q))
    wait([out_cp(i) for i in range(3, NB - 1)] + sum([last_cp(q) for q in range(4)], []))


@jax.jit
def pallas_parallel_sum__ssm_conv_s5__moe_arch_mod__prompt_kernel(
    A_x, A_Lambda_re, A_Lambda_im, A_B_re, A_B_im, A_C_re, A_C_im, A_log_dt, A_Dskip,
    B_x, B_w_r, B_w_gate, B_w_up, B_w_down,
):
    hbm = pl.BlockSpec(memory_space=pl.ANY)
    vm = pl.BlockSpec(memory_space=pltpu.VMEM)
    out = pl.pallas_call(
        _kernel,
        out_shape=jax.ShapeDtypeStruct((L, D), f32),
        in_specs=[hbm, vm, vm, hbm, hbm, hbm, hbm, vm, vm, vm, hbm, hbm, hbm],
        out_specs=hbm,
        scratch_shapes=[
            pltpu.VMEM((L, D), bf16), pltpu.VMEM((G, NB * TP, 128), f32),
            pltpu.VMEM((L, D), f32), pltpu.VMEM((G, TP, 128), f32),
            pltpu.VMEM((2, P, D), bf16), pltpu.VMEM((2, D, P), bf16),
            pltpu.VMEM((7, P, D // 2), bf16), pltpu.VMEM((7, D // 2, P), bf16),
            pltpu.VMEM((D, F), bf16), pltpu.VMEM((D, F), bf16), pltpu.VMEM((F, D), bf16),
            pltpu.VMEM((J, 128), f32), pltpu.VMEM((10, 8, P), f32),
            pltpu.SemaphoreType.DMA((NB + 5 + 2 * NC,)), pltpu.SemaphoreType.DMA((NB + 7,)),
            *[pltpu.VMEM((7, T // 2, D // 2), bf16)] * 4,
            *[pltpu.VMEM((2, 2, T // 2, P), f32)] * 3,
            *[pltpu.VMEM((7, T // 2, P), bf16)] * 3,
        ],
        compiler_params=pltpu.CompilerParams(
            vmem_limit_bytes=110 * 1024 * 1024,
            flags={'XLA_TPU_EVENLY_DISTRIBUTE_CRITICAL_NODES': True}),
    )(A_x.reshape(L, D), A_Lambda_re, A_Lambda_im, A_B_re, A_B_im, A_C_re, A_C_im,
      A_log_dt, A_Dskip, B_w_r, B_w_gate, B_w_up, B_w_down)
    return out.reshape(1, L, D)
```
